```python
import os as _os
_os.environ.setdefault("JAX_PLATFORMS", "cpu")
import jax
import jax.numpy as jnp

def _softmax(x, axis=-1):
    return jax.nn.softmax(x, axis=axis)
def _gelu(x):
    return jax.nn.gelu(x, approximate=True)
def _silu(x):
    return jax.nn.silu(x)
def _sigmoid(x):
    return jax.nn.sigmoid(x)
def _layernorm(x, axis=-1, eps=1e-5):
    m = jnp.mean(x, axis=axis, keepdims=True)
    v = jnp.var(x, axis=axis, keepdims=True)
    return (x - m) / jnp.sqrt(v + eps)
def _scatter_add(tgt, idx, src, axis=0):
    return tgt.at[idx].add(src)
def _segment_sum(src, seg, n):
    return jax.ops.segment_sum(src, seg, n)
class _Rng:
    def __init__(self, key):
        self._k = key
    def _next(self):
        self._k, sub = jax.random.split(self._k)
        return sub
    def normal(self, shape):
        return jax.random.normal(self._next(), shape, dtype=jnp.bfloat16)
    def randint(self, lo, hi, shape):
        return jax.random.randint(self._next(), shape, lo, hi, dtype=jnp.int32)
    def uniform(self, shape, lo=0.0, hi=1.0):
        return jax.random.uniform(self._next(), shape, jnp.bfloat16, lo, hi)
    def permutation(self, n):
        return jax.random.permutation(self._next(), n)


kernel_name = 'interleave_layers__softmax_full_mha__glu_gated_bilinear__prompt'

def setup_inputs():
    _rng = _Rng(jax.random.key(int.from_bytes(__import__("os").urandom(4), "little")))
    _w = (lambda a: (lambda t: t.astype(jnp.bfloat16) if jnp.issubdtype(t.dtype, jnp.floating) else t)(jnp.asarray(a)))
    def _A_setup():
        B, S, D = 1, 2048, 512
        return {
            "x": _w((lambda *s: _rng.normal(s) * 0.05)(B, S, D)),
            "wqkv": _w((lambda *s: _rng.normal(s) * 0.05)(D, 3 * D)),
            "wo": _w((lambda *s: _rng.normal(s) * 0.05)(D, D)),
        }
    _A_in = _A_setup()

    def _B_setup():
        B, S, D, F = 1, 2048, 512, 1792
        return {
            "x": _w((lambda *s: _rng.normal(s) * 0.05)(B, S, D)),
            "w_gate": _w((lambda *s: _rng.normal(s) * 0.4)(D, F) * (D ** -0.5)),
            "w_up": _w((lambda *s: _rng.normal(s) * 0.4)(D, F) * (D ** -0.5)),
            "w_down": _w((lambda *s: _rng.normal(s) * 0.4)(F, D) * (F ** -0.5)),
        }
    _B_in = _B_setup()

    return {
        "A_x": _A_in["x"],
        "A_wqkv": _A_in["wqkv"],
        "A_wo": _A_in["wo"],
        "B_x": _B_in["x"],
        "B_w_gate": _B_in["w_gate"],
        "B_w_up": _B_in["w_up"],
        "B_w_down": _B_in["w_down"],
    }

def reference(A_x, A_wqkv, A_wo, B_x, B_w_gate, B_w_up, B_w_down):
    def _A_ref(x, wqkv, wo):
        B, S, D = x.shape
        H = 32; Dh = D // H
        qkv = (lambda x, *d: x.transpose(*d))((x @ wqkv).reshape(B, S, 3, H, Dh), 2, 0, 3, 1, 4)
        q, k, v = qkv[0], qkv[1], qkv[2]
        scale = Dh ** -0.5
        scores = jnp.einsum("bhqd,bhkd->bhqk", q, k) * scale
        p = _softmax(scores, axis=-1)
        o = jnp.einsum("bhqk,bhkd->bhqd", p, v)
        return (lambda x, *d: x.transpose(*d))(o, 0, 2, 1, 3).reshape(B, S, D) @ wo

    def _B_ref(x, w_gate, w_up, w_down):
        g = jnp.einsum("bsd,df->bsf", x, w_gate)
        u = jnp.einsum("bsd,df->bsf", x, w_up)
        h = g * u
        return jnp.einsum("bsf,fd->bsd", h, w_down)

    x = A_x
    x = x + _A_ref(_layernorm(x, axis=-1), A_wqkv, A_wo)
    x = x + _B_ref(_layernorm(x, axis=-1), B_w_gate, B_w_up, B_w_down)
    x = x + _A_ref(_layernorm(x, axis=-1), A_wqkv, A_wo)
    x = x + _B_ref(_layernorm(x, axis=-1), B_w_gate, B_w_up, B_w_down)
    return x
```

```python
import functools
import math

import jax
import jax.numpy as jnp
from jax import lax
import jax.experimental.pallas as pl
import jax.experimental.pallas.tpu as pltpu

S, D, H, DH, F = 2048, 512, 32, 16, 1792
EPS = 1e-5
BF16 = jnp.bfloat16
F32 = jnp.float32


def _ln(x):
    m = jnp.mean(x, axis=-1, keepdims=True)
    xc = x - m
    v = jnp.mean(xc * xc, axis=-1, keepdims=True)
    return xc * lax.rsqrt(v + EPS)


def make(TQ=512, CK=128, G=4, TMA=512, TMC=256, FC=1792, phases="ABC"):
    nq = S // TQ
    nc = S // CK
    NU = H * nq // G
    qscale = (DH ** -0.5) * math.log2(math.e)

    def kernel(x_ref, wqkv_ref, wo_ref, wg_ref, wu_ref, wd_ref, o_ref,
               x_s, wqvT_s, k_s, qT_s, vT_s, oT_s, s_s, m_s):
        x_s[...] = x_ref[...].astype(F32)
        wqvT_s[0:D, :] = wqkv_ref[:, 0:D].astype(F32).T.astype(BF16)
        wqvT_s[D:2 * D, :] = wqkv_ref[:, 2 * D:3 * D].astype(F32).T.astype(BF16)

        def phase_a(r, carry):
            rows = pl.ds(pl.multiple_of(r * TMA, TMA), TMA)
            xn = _ln(x_s[rows, :]).astype(BF16)
            kk = jnp.dot(xn, wqkv_ref[:, D:2 * D], preferred_element_type=F32).astype(BF16)
            for g in range(4):
                k_s[g, rows, :] = kk[:, g * 128:(g + 1) * 128]
            qv = lax.dot_general(wqvT_s[...], xn, (((1,), (1,)), ((), ())), preferred_element_type=F32)
            qT_s[:, rows] = (qv[0:D] * qscale).astype(BF16)
            vT_s[:, rows] = qv[D:2 * D].astype(BF16)
            return carry

        def qmask(h, hh, qoff):
            if isinstance(hh, int):
                qh = qT_s[pl.ds(pl.multiple_of(h * DH, DH), DH), pl.ds(qoff, TQ)]
                parts = []
                if hh > 0:
                    parts.append(jnp.zeros((DH * hh, TQ), BF16))
                parts.append(qh)
                if hh < 7:
                    parts.append(jnp.zeros((DH * (7 - hh), TQ), BF16))
                return jnp.concatenate(parts, axis=0)
            g = h // 8
            qg = qT_s[pl.ds(pl.multiple_of(g * 128, 128), 128), pl.ds(qoff, TQ)]
            rows = lax.broadcasted_iota(jnp.int32, (128, TQ), 0)
            return jnp.where((rows // DH) == hh, qg, jnp.zeros_like(qg))

        def unit(n):
            per = 8 // G
            return n // (per * nq), (n // per) % nq, (n % per) * G

        def mo(v, m):
            return v if isinstance(v, int) else pl.multiple_of(v, m)

        def att_step(n1, n2):
            for e in range(G):
                m8 = None
                l8 = None
                acc = None
                if n1 is not None:
                    g1, j1, hb1 = unit(n1)
                    hh1 = e if G == 8 else hb1 + e
                    qm = qmask(g1 * 8 + hh1, hh1, mo(j1 * TQ, TQ))
                if n2 is not None:
                    g2, j2, hb2 = unit(n2)
                    h2 = g2 * 8 + hb2 + e
                    hrows = pl.ds(mo(h2 * DH, DH), DH)
                    mb = jnp.broadcast_to(m_s[e], (8, TQ))
                for c in range(nc):
                    sl = slice(c * CK, (c + 1) * CK)
                    if n2 is not None:
                        sp = s_s[e, sl, :].reshape(CK // 8, 8, TQ)
                        p = jnp.exp2(sp - mb[None])
                        lc = jnp.sum(p, axis=0)
                        l8 = lc if l8 is None else l8 + lc
                        pb = p.reshape(CK, TQ).astype(BF16)
                        a = jnp.dot(vT_s[hrows, sl], pb, preferred_element_type=F32)
                        acc = a if acc is None else acc + a
                    if n1 is not None:
                        sT = jnp.dot(k_s[g1, sl, :], qm, preferred_element_type=F32)
                        s_s[e, sl, :] = sT
                        mc = jnp.max(sT.reshape(CK // 8, 8, TQ), axis=0)
                        m8 = mc if m8 is None else jnp.maximum(m8, mc)
                if n2 is not None:
                    l = jnp.sum(l8, axis=0, keepdims=True)
                    oT_s[hrows, pl.ds(mo(j2 * TQ, TQ), TQ)] = (acc * (1.0 / l)).astype(BF16)
                if n1 is not None:
                    m_s[e] = jnp.max(m8, axis=0, keepdims=True)

        def phase_b():
            att_step(0, None)

            def body(it, carry):
                att_step(it + 1, it)
                return carry
            lax.fori_loop(0, NU - 1, body, 0)
            att_step(None, NU - 1)

        def phase_c(r, carry):
            rows = pl.ds(pl.multiple_of(r * TMC, TMC), TMC)
            attn = lax.dot_general(oT_s[:, rows], wo_ref[...], (((0,), (0,)), ((), ())),
                                   preferred_element_type=F32)
            x1 = x_s[rows, :] + attn
            xn = _ln(x1).astype(BF16)
            y = x1
            for f in range(F // FC):
                fs = slice(f * FC, (f + 1) * FC)
                g = jnp.dot(xn, wg_ref[:, fs], preferred_element_type=F32)
                u = jnp.dot(xn, wu_ref[:, fs], preferred_element_type=F32)
                hh = (g * u).astype(BF16)
                y = y + jnp.dot(hh, wd_ref[fs, :], preferred_element_type=F32)
            x_s[rows, :] = y
            return carry

        def layer(_, carry):
            if "A" in phases:
                lax.fori_loop(0, S // TMA, phase_a, 0)
            if "B" in phases:
                phase_b()
            if "C" in phases:
                lax.fori_loop(0, S // TMC, phase_c, 0)
            return carry

        lax.fori_loop(0, 2, layer, 0)
        o_ref[...] = x_s[...].astype(o_ref.dtype)

    @jax.jit
    def run(A_x, A_wqkv, A_wo, B_x, B_w_gate, B_w_up, B_w_down):
        x = A_x.reshape(S, D)
        out = pl.pallas_call(
            kernel,
            out_shape=jax.ShapeDtypeStruct((S, D), A_x.dtype),
            scratch_shapes=[
                pltpu.VMEM((S, D), F32),
                pltpu.VMEM((2 * D, D), BF16),
                pltpu.VMEM((4, S, 128), BF16),
                pltpu.VMEM((D, S), BF16),
                pltpu.VMEM((D, S), BF16),
                pltpu.VMEM((D, S), BF16),
                pltpu.VMEM((G, S, TQ), F32),
                pltpu.VMEM((G, 1, TQ), F32),
            ],
            compiler_params=pltpu.CompilerParams(vmem_limit_bytes=110 * 1024 * 1024),
        )(x, A_wqkv, A_wo, B_w_gate, B_w_up, B_w_down)
        return out.reshape(1, S, D)
    return run


_run = make()


def pallas_interleave_layers__softmax_full_mha__glu_gated_bilinear__prompt_kernel(
    A_x, A_wqkv, A_wo, B_x, B_w_gate, B_w_up, B_w_down
):
    return _run(A_x, A_wqkv, A_wo, B_x, B_w_gate, B_w_up, B_w_down)
```

```python
import functools
import math

import jax
import jax.numpy as jnp
from jax import lax
import jax.experimental.pallas as pl
import jax.experimental.pallas.tpu as pltpu

S, D, H, DH, F = 2048, 512, 32, 16, 1792
EPS = 1e-5
BF16 = jnp.bfloat16
F32 = jnp.float32
TQ = 512
CK = 128
NT = TQ // 128
NC = S // CK
NB = (H // 8) * (S // TQ)


def _ln(x):
    m = jnp.mean(x, axis=-1, keepdims=True)
    xc = x - m
    v = jnp.mean(xc * xc, axis=-1, keepdims=True)
    return xc * lax.rsqrt(v + EPS)


def _mo(v, m):
    return v if isinstance(v, int) else pl.multiple_of(v, m)


def make(pattern="1111111111000000", NROT=2, vlag=1, TMA=512, TMC=256, x0order=0):
    qscale = (DH ** -0.5) * math.log2(math.e)
    vr = [16 * int(ch) for ch in pattern]
    KV = sum(vr)
    HPR = 8 // NROT
    items = [(i, (i + 1) * CK - vr[i] + r) for i in range(NC) for r in range(0, vr[i], 8)]
    NA = S // TMA
    NCT = S // TMC

    def kernel(x_hbm, wqkv_hbm, wo_hbm, wg_hbm, wu_hbm, wd_hbm, o_hbm,
               xin_s, wqkv_ref, wo_ref, wg_ref, wu_ref, wd_ref, out_s,
               x_s, xa_s, xn_s, wqvT_s, k_s, kf_s, qT_s, qf_s, vT_s, oT_s, s_s, m_s, l_s, zs,
               sem_x, sem_w, sem_o):
        def x_copy(t):
            rows = pl.ds(_mo(t * TMA, TMA), TMA)
            return pltpu.make_async_copy(x_hbm.at[rows, :], xin_s.at[rows, :], sem_x.at[t])

        w_pairs = ((wqkv_hbm, wqkv_ref), (wo_hbm, wo_ref), (wg_hbm, wg_ref), (wu_hbm, wu_ref), (wd_hbm, wd_ref))

        def w_copy(i):
            return pltpu.make_async_copy(w_pairs[i][0], w_pairs[i][1], sem_w.at[i])

        def o_copy(t):
            rows = pl.ds(_mo(t * TMC, TMC), TMC)
            return pltpu.make_async_copy(out_s.at[rows, :], o_hbm.at[rows, :], sem_o.at[t])

        w_copy(0).start()
        x_copy(0).start()
        for i in range(max(len(items), 1)):
            zs[i] = 0
        w_copy(0).wait()
        for t in range(1, NA):
            x_copy(t).start()
        wqvT_s[0:D, :] = wqkv_ref[:, 0:D].astype(F32).T.astype(BF16)
        wqvT_s[D:2 * D, :] = wqkv_ref[:, 2 * D:3 * D].astype(F32).T.astype(BF16)
        x_copy(0).wait()
        for i in range(1, 5):
            w_copy(i).start()
        x0 = xin_s[0:TMA, :].astype(F32)
        x_s[0:TMA, :] = x0
        xa_s[...] = _ln(x0).astype(BF16)

        def phase_a(t, xn, first):
            tn = jnp.minimum(t + 1, NA - 1)

            @pl.when(jnp.logical_and(first, t + 1 < NA))
            def _():
                x_copy(tn).wait()

            rows = pl.ds(pl.multiple_of(t * TMA, TMA), TMA)
            kk = jnp.dot(xn, wqkv_ref[:, D:2 * D], preferred_element_type=F32)
            for g in range(4):
                kg = kk[:, g * 128:(g + 1) * 128]
                kf_s[g, rows, :] = kg
                for r in range(NROT):
                    k_s[r, g, rows, :] = (kg if r == 0 else pltpu.roll(kg, 128 - r * HPR * DH, 1)).astype(BF16)
            qv = lax.dot_general(wqvT_s[...], xn, (((1,), (1,)), ((), ())), preferred_element_type=F32)
            q = qv[0:D] * qscale
            qT_s[:, rows] = q.astype(BF16)
            for c in range(TMA // 128):
                qf_s[t * (TMA // 128) + c] = q[:, c * 128:(c + 1) * 128]
            vT_s[:, rows] = qv[D:2 * D]
            nrows = pl.ds(pl.multiple_of(tn * TMA, TMA), TMA)
            xv = jnp.where(first, xin_s[nrows, :].astype(F32), x_s[nrows, :])
            x_s[nrows, :] = xv
            return _ln(xv).astype(BF16)

        def qmask(h, hp, j):
            qh = qT_s[pl.ds(_mo(h * DH, DH), DH), pl.ds(_mo(j * TQ, TQ), TQ)]
            parts = []
            if hp > 0:
                parts.append(jnp.zeros((DH * hp, TQ), BF16))
            parts.append(qh)
            if hp < 7:
                parts.append(jnp.zeros((DH * (7 - hp), TQ), BF16))
            return jnp.concatenate(parts, axis=0)

        def att_unit(b1, b2, hh, pieces=None):
            l8 = None
            acc = None
            m8 = [None] * NT
            if b2 is not None:
                g2, j2 = b2 % 4, b2 // 4
                mb = jnp.broadcast_to(m_s[hh], (8, TQ))
                hrows = pl.ds(_mo((g2 * 8 + hh) * DH, DH), DH)
            if b1 is not None:
                g1, j1 = b1 % 4, b1 // 4
                qm = qmask(g1 * 8 + hh, hh % HPR, j1)

            def upd(t, x):
                m8[t] = x if m8[t] is None else jnp.maximum(m8[t], x)

            def v_item(r0, idx):
                zz = zs[idx]
                kf = kf_s[g1 + zz, r0:r0 + 8, :]
                svs = [None] * NT
                for d in range(DH):
                    col = hh * DH + d
                    kb = jnp.broadcast_to(kf[:, col:col + 1], (8, 128))
                    for w in range(NT):
                        qd = qf_s[(j1 + zz) * NT + w, pl.ds((g1 * 8 + hh) * DH + d, 8, stride=0), :]
                        tt = kb * qd
                        svs[w] = tt if svs[w] is None else svs[w] + tt
                for w in range(NT):
                    s_s[hh, r0:r0 + 8, w * 128:(w + 1) * 128] = svs[w]
                    upd(w, svs[w])

            tot_rg = (S - KV) // 8
            lag_rg = vlag * 16
            rg_done = 0
            vdone = 0
            for i in range(NC):
                sl = slice(i * CK, (i + 1) * CK)
                if pieces is not None and i % 2 == 0:
                    next(pieces, None)
                if b2 is not None:
                    sp = s_s[hh, sl, :].reshape(CK // 8, 8, TQ)
                    p = jnp.exp2(sp - mb[None])
                    for r in range(CK // 8 - 1, -1, -1):
                        l8 = p[r] if l8 is None else l8 + p[r]
                    a = jnp.dot(vT_s[hrows, sl], p.reshape(CK, TQ), preferred_element_type=F32)
                    acc = a if acc is None else a + acc
                if b1 is not None:
                    lo, hi = i * CK, (i + 1) * CK - vr[i]
                    sT = jnp.dot(k_s[hh // HPR, g1, lo:hi, :], qm, preferred_element_type=F32)
                    s_s[hh, lo:hi, :] = sT
                    for r in range((hi - lo) // 8):
                        for t in range(NT):
                            upd(t, sT[r * 8:(r + 1) * 8, t * 128:(t + 1) * 128])
                        rg_done += 1
                        want = max(0, rg_done - lag_rg) * len(items) // (tot_rg - lag_rg)
                        while vdone < want and items[vdone][0] <= i:
                            v_item(items[vdone][1], vdone)
                            vdone += 1
            if b2 is not None:
                l = jnp.sum(l8, axis=0, keepdims=True)
                oT_s[hrows, pl.ds(_mo(j2 * TQ, TQ), TQ)] = (acc * (1.0 / l)).astype(BF16)
            if b1 is not None:
                assert vdone == len(items)
                m_s[hh] = jnp.max(jnp.concatenate(m8, axis=1), axis=0, keepdims=True)

        def c1(r0, n):
            rows = slice(r0, r0 + n)
            attn = lax.dot_general(oT_s[:, rows], wo_ref[...], (((0,), (0,)), ((), ())),
                                   preferred_element_type=F32)
            x1 = x_s[rows, :] + attn
            x_s[rows, :] = x1
            xn_s[rows, :] = _ln(x1).astype(BF16)

        def c2(t, last):
            rows = pl.ds(_mo(t * TMC, TMC), TMC)
            xn = xn_s[rows, :]
            g = jnp.dot(xn, wg_ref[...], preferred_element_type=F32)
            u = jnp.dot(xn, wu_ref[...], preferred_element_type=F32)
            hh = (g * u).astype(BF16)
            y = x_s[rows, :] + jnp.dot(hh, wd_ref[...], preferred_element_type=F32)
            x_s[rows, :] = y
            out_s[rows, :] = y.astype(BF16)

        def start_out(t, last):
            @pl.when(last)
            def _():
                o_copy(t).start()

        def dense_pieces():
            for rb in range((S - TQ) // TMC):
                rows = slice(rb * TMC, (rb + 1) * TMC)
                o = oT_s[:, rows].T
                cols = []
                for c in range(D // 128):
                    cols.append(jnp.dot(o, wo_ref[:, c * 128:(c + 1) * 128], preferred_element_type=F32))
                    if c == D // 128 - 1:
                        x1 = x_s[rows, :] + jnp.concatenate(cols, axis=1)
                        x_s[rows, :] = x1
                        xn_s[rows, :] = _ln(x1).astype(BF16)
                    yield
            rows = slice(0, TMC)
            y = None
            hs = []
            for f in range(F // 128):
                fs = slice(f * 128, (f + 1) * 128)
                g = jnp.dot(xn_s[rows, :], wg_ref[:, fs], preferred_element_type=F32)
                yield
                u = jnp.dot(xn_s[rows, :], wu_ref[:, fs], preferred_element_type=F32)
                hs.append((g * u).astype(BF16))
                yield
                if f >= 1:
                    a = jnp.dot(hs[f - 1], wd_ref[(f - 1) * 128:f * 128, :], preferred_element_type=F32)
                    y = a if y is None else a + y
                    yield
            a = jnp.dot(hs[-1], wd_ref[F - 128:F, :], preferred_element_type=F32)
            y = x_s[rows, :] + (a + y)
            x_s[rows, :] = y
            out_s[rows, :] = y.astype(BF16)
            yield

        def layer(li, carry):
            first = li == 0
            last = li == 1
            lax.fori_loop(0, NA, functools.partial(phase_a, first=first), xa_s[...])
            for hh in range(8):
                att_unit(0, None, hh)

            def body(b, c):
                for hh in range(8):
                    att_unit(b + 1, b, hh)
                return c
            lax.fori_loop(0, NB - 1, body, 0)

            @pl.when(first)
            def _():
                for i in range(1, 5):
                    w_copy(i).wait()

            pieces = dense_pieces()
            for hh in range(8):
                att_unit(None, NB - 1, hh, pieces)
            for _ in pieces:
                pass
            start_out(0, last)

            def x1blk(_, c):
                c1(S - TQ, TQ)
                c2(1, last)
                start_out(1, last)
                return c
            lax.fori_loop(0, 1 + zs[0], x1blk, 0)

            def cbody(t, c):
                piece = jnp.minimum(t - 2, TMA // 128 - 1)
                prow = pl.ds(pl.multiple_of(piece * 128, 128), 128)
                xa_s[prow, :] = _ln(x_s[prow, :]).astype(BF16)
                c2(t, last)
                start_out(t, last)
                return c
            lax.fori_loop(2, NCT, cbody, 0)
            return carry

        lax.fori_loop(0, 2, layer, 0)
        for t in range(NCT):
            o_copy(t).wait()

    @jax.jit
    def run(A_x, A_wqkv, A_wo, B_x, B_w_gate, B_w_up, B_w_down):
        x = A_x.reshape(S, D)
        out = pl.pallas_call(
            kernel,
            out_shape=jax.ShapeDtypeStruct((S, D), A_x.dtype),
            in_specs=[pl.BlockSpec(memory_space=pl.ANY)] * 6,
            out_specs=pl.BlockSpec(memory_space=pl.ANY),
            scratch_shapes=[
                pltpu.VMEM((S, D), BF16),
                pltpu.VMEM((D, 3 * D), BF16),
                pltpu.VMEM((D, D), BF16),
                pltpu.VMEM((D, F), BF16),
                pltpu.VMEM((D, F), BF16),
                pltpu.VMEM((F, D), BF16),
                pltpu.VMEM((S, D), BF16),
                pltpu.VMEM((S, D), F32),
                pltpu.VMEM((TMA, D), BF16),
                pltpu.VMEM((S, D), BF16),
                pltpu.VMEM((2 * D, D), BF16),
                pltpu.VMEM((NROT, 4, S, 128), BF16),
                pltpu.VMEM((4, S, 128), F32),
                pltpu.VMEM((D, S), BF16),
                pltpu.VMEM((S // 128, D, 128), F32),
                pltpu.VMEM((D, S), F32),
                pltpu.VMEM((D, S), BF16),
                pltpu.VMEM((8, S, TQ), F32),
                pltpu.VMEM((8, 1, TQ), F32),
                pltpu.VMEM((8, 1, TQ), F32),
                pltpu.SMEM((64,), jnp.int32),
                pltpu.SemaphoreType.DMA((NA,)),
                pltpu.SemaphoreType.DMA((5,)),
                pltpu.SemaphoreType.DMA((NCT,)),
            ],
            compiler_params=pltpu.CompilerParams(vmem_limit_bytes=120 * 1024 * 1024),
        )(x, A_wqkv, A_wo, B_w_gate, B_w_up, B_w_down)
        return out.reshape(1, S, D)
    return run


_run = make()


def pallas_interleave_layers__softmax_full_mha__glu_gated_bilinear__prompt_kernel(
    A_x, A_wqkv, A_wo, B_x, B_w_gate, B_w_up, B_w_down
):
    return _run(A_x, A_wqkv, A_wo, B_x, B_w_gate, B_w_up, B_w_down)
```

```python
import functools
import math

import jax
import jax.numpy as jnp
from jax import lax
import jax.experimental.pallas as pl
import jax.experimental.pallas.tpu as pltpu

S, D, H, DH, F = 2048, 512, 32, 16, 1792
EPS = 1e-5
BF16 = jnp.bfloat16
F32 = jnp.float32
TQ = 512
CK = 128
NT = TQ // 128
NC = S // CK
NB = (H // 8) * (S // TQ)
TMA = 512
NA = S // TMA
TM0 = 256


def _ln(x):
    m = jnp.mean(x, axis=-1, keepdims=True)
    xc = x - m
    v = jnp.mean(xc * xc, axis=-1, keepdims=True)
    return xc * lax.rsqrt(v + EPS)


def _mo(v, m):
    return v if isinstance(v, int) else pl.multiple_of(v, m)


def make(pattern="1111111111110000", pattern0="2111211121112110", NROT=4, vlag=0, TMC=256, c1pos=14, aorder=0, split_ab=2, only=None, shift=0, ku32=1, anti=0):
    qscale = (DH ** -0.5) * math.log2(math.e)
    HPR = 8 // NROT
    assert pattern[-1] == '0' and pattern0[-1] == '0'
    NCL = (S - 2 * TM0) // TMC
    out_tiles = [(0, TM0), (TM0, TM0)] + [(2 * TM0 + t * TMC, TMC) for t in range(NCL)]

    def kernel(x_hbm, wqkv_hbm, wo_hbm, wg_hbm, wu_hbm, wd_hbm, o_hbm,
               xin_s, wqkv_ref, wo_ref, wg_ref, wu_ref, wd_ref, out_s,
               x_s, xa_s, xn_s, wqvT_s, k_s, kf_s, qT_s, qf_s, vT_s, oT_s, s_s, m_s, mp_s,
               sem_x, sem_w, sem_o):
        def x_copy(t):
            rows = slice(0, TMA) if t == 0 else slice(TMA, S)
            return pltpu.make_async_copy(x_hbm.at[rows, :], xin_s.at[rows, :], sem_x.at[t])

        w_pairs = ((wqkv_hbm, wqkv_ref), (wo_hbm, wo_ref), (wg_hbm, wg_ref), (wu_hbm, wu_ref), (wd_hbm, wd_ref))

        def w_copy(i):
            return pltpu.make_async_copy(w_pairs[i][0], w_pairs[i][1], sem_w.at[i])

        def o_copy(i, r0, n):
            rows = pl.ds(r0, n)
            return pltpu.make_async_copy(out_s.at[rows, :], o_hbm.at[rows, :], sem_o.at[i])

        x_copy(0).start()
        w_copy(0).start()
        x_copy(0).wait()
        x0 = xin_s[0:TMA, :].astype(F32)
        x_s[0:TMA, :] = x0
        xa_s[...] = _ln(x0).astype(BF16)
        w_copy(0).wait()
        x_copy(1).start()
        wqT = wqkv_ref[:, 0:D].astype(F32).T.astype(BF16)
        wvT = wqkv_ref[:, 2 * D:3 * D].astype(F32).T.astype(BF16)
        for h in range(H):
            wqvT_s[2 * h * DH:(2 * h + 1) * DH, :] = wqT[h * DH:(h + 1) * DH]
            wqvT_s[(2 * h + 1) * DH:(2 * h + 2) * DH, :] = wvT[h * DH:(h + 1) * DH]

        def proj_k(t, xn):
            rows = slice(t * TMA, (t + 1) * TMA)
            kk = jnp.dot(xn, wqkv_ref[:, D:2 * D], preferred_element_type=F32)
            for g in range(4):
                kg = kk[:, g * 128:(g + 1) * 128]
                kf_s[g, rows, :] = kg
                for r in range(NROT):
                    kb16 = (kg if r == 0 else pltpu.roll(kg, 128 - r * HPR * DH, 1)).astype(BF16)
                    if ku32:
                        k_s[r, g, t * TMA // 2:(t + 1) * TMA // 2, :] = pltpu.bitcast(kb16, jnp.uint32)
                    else:
                        k_s[r, g, rows, :] = kb16

        def proj_qv(t, xn):
            rows = slice(t * TMA, (t + 1) * TMA)
            qv = lax.dot_general(wqvT_s[...], xn, (((1,), (1,)), ((), ())), preferred_element_type=F32)
            qv = qv.reshape(H, 2 * DH, TMA)
            q = qv[:, 0:DH, :].reshape(D, TMA) * qscale
            qT_s[:, rows] = q.astype(BF16)
            for c in range(TMA // 128):
                qc = q[:, c * 128:(c + 1) * 128]
                qf_s[t * (TMA // 128) + c] = jnp.broadcast_to(qc[:, None, :], (D, 8, 128))
            vT_s[:, rows] = qv[:, DH:2 * DH, :].reshape(D, TMA)

        def phase_a(first):
            def ln_tile(t):
                rows = slice(t * TMA, (t + 1) * TMA)
                xv = jnp.where(first, xin_s[rows, :].astype(F32), x_s[rows, :])
                x_s[rows, :] = xv
                xn_s[rows, :] = _ln(xv).astype(BF16)

            proj_k(0, xa_s[...])

            @pl.when(first)
            def _():
                x_copy(1).wait()
                for i in range(1, 5):
                    w_copy(i).start()

            ln_tile(1)
            proj_qv(0, xa_s[...])
            for t in range(1, NA):
                rows = slice(t * TMA, (t + 1) * TMA)
                if t + 1 < NA:
                    ln_tile(t + 1)
                proj_k(t, xn_s[rows, :])
                if aorder == 0:
                    proj_qv(t, xn_s[rows, :])
            if aorder == 1:
                for t in range(1, NA):
                    proj_qv(t, xn_s[t * TMA:(t + 1) * TMA, :])

        def k_rows(r, g, lo, hi):
            if ku32:
                return pltpu.bitcast(k_s[r, g, lo // 2:hi // 2, :], BF16)
            return k_s[r, g, lo:hi, :]

        def qmask(h, hp, j):
            qh = qT_s[pl.ds(_mo(h * DH, DH), DH), pl.ds(_mo(j * TQ, TQ), TQ)]
            parts = []
            if hp > 0:
                parts.append(jnp.zeros((DH * hp, TQ), BF16))
            parts.append(qh)
            if hp < 7:
                parts.append(jnp.zeros((DH * (7 - hp), TQ), BF16))
            return jnp.concatenate(parts, axis=0)

        def att_unit(b1, b2, hh, pat, pieces=None):
            vr = [16 * int(ch) for ch in pat]
            KV = sum(vr)
            items = [(i, (i + 1) * CK - vr[i] + r) for i in range(NC) for r in range(0, vr[i], 8)]
            l8 = None
            acc = None
            m8 = [None] * NT
            if b2 is not None:
                g2, j2 = b2 % 4, b2 // 4
                mb = jnp.broadcast_to(m_s[hh], (8, TQ))
                hrows = pl.ds(_mo((g2 * 8 + hh) * DH, DH), DH)
            if b1 is not None:
                g1, j1 = b1 % 4, b1 // 4
                qm = qmask(g1 * 8 + hh, hh % HPR, j1)

            def upd(t, x):
                m8[t] = x if m8[t] is None else jnp.maximum(m8[t], x)

            def v_item(r0, idx):
                zz = lax.shift_right_logical(b1, 5 + idx % 26)
                kf = kf_s[g1 + zz, r0:r0 + 8, :]
                lane = lax.broadcasted_iota(jnp.int32, (8, 128), 1)
                svs = [None] * NT
                for d in range(DH):
                    col = hh * DH + d
                    kb = jnp.broadcast_to(jnp.sum(jnp.where(lane == col, kf, 0.0), axis=1, keepdims=True), (8, 128))
                    for w in range(NT):
                        qd = qf_s[(j1 + zz) * NT + w, (g1 * 8 + hh) * DH + d]
                        tt = kb * qd
                        svs[w] = tt if svs[w] is None else svs[w] + tt
                for w in range(NT):
                    s_s[hh, r0:r0 + 8, w * 128:(w + 1) * 128] = svs[w]
                    upd(w, svs[w])

            tot_rg = (S - KV) // 8
            if shift and hh == 7:
                tot_rg -= (CK - vr[NC - 1]) // 8
            lag_rg = vlag * 16
            rg_done = 0
            vdone = 0
            for i in range(NC):
                sl = slice(i * CK, (i + 1) * CK)
                if pieces is not None and i % 2 == 0:
                    next(pieces, None)
                if b2 is not None:
                    sp = s_s[hh, sl, :].reshape(CK // 8, 8, TQ)
                    p = jnp.exp2(sp - mb[None])
                    for r in range(CK // 8 - 1, -1, -1):
                        l8 = p[r] if l8 is None else l8 + p[r]
                    a = jnp.dot(vT_s[hrows, sl], p.reshape(CK, TQ), preferred_element_type=F32)
                    acc = a if acc is None else a + acc
                if b1 is not None and not (shift and hh == 7 and i == NC - 1):
                    lo, hi = i * CK, (i + 1) * CK - vr[i]
                    sT = jnp.dot(k_rows(hh // HPR, g1, lo, hi), qm, preferred_element_type=F32)
                    s_s[hh, lo:hi, :] = sT
                    for r in range((hi - lo) // 8):
                        for t in range(NT):
                            upd(t, sT[r * 8:(r + 1) * 8, t * 128:(t + 1) * 128])
                        rg_done += 1
                        want = max(0, rg_done - lag_rg) * len(items) // (tot_rg - lag_rg)
                        while vdone < want and (b2 is None or items[vdone][0] <= i):
                            v_item(items[vdone][1], vdone)
                            vdone += 1
            if b2 is not None:
                l = jnp.sum(l8, axis=0, keepdims=True)
                oT_s[hrows, pl.ds(_mo(j2 * TQ, TQ), TQ)] = (acc * (1.0 / l)).astype(BF16)
            if b1 is not None:
                assert vdone == len(items)
                if shift and hh == 7:
                    mp_s[...] = jnp.concatenate(m8, axis=1)
                else:
                    m_s[hh] = jnp.max(jnp.concatenate(m8, axis=1), axis=0, keepdims=True)

        def s1_tail(b, nrows):
            g, j = b % 4, b // 4
            lo = (NC - 1) * CK
            sT = jnp.dot(k_rows(7 // HPR, g, lo, lo + nrows), qmask(g * 8 + 7, 7 % HPR, j), preferred_element_type=F32)
            s_s[7, lo:lo + nrows, :] = sT
            mm = jnp.maximum(mp_s[...], jnp.max(sT.reshape(nrows // 8, 8, TQ), axis=0))
            m_s[7] = jnp.max(mm, axis=0, keepdims=True)

        def c1_pieces(rb):
            rows = slice(rb * TM0, (rb + 1) * TM0)
            o = oT_s[:, rows].T
            cols = []
            for c in range(D // 128):
                cols.append(jnp.dot(o, wo_ref[:, c * 128:(c + 1) * 128], preferred_element_type=F32))
                if c == D // 128 - 1:
                    x1 = x_s[rows, :] + jnp.concatenate(cols, axis=1)
                    x_s[rows, :] = x1
                    xn_s[rows, :] = _ln(x1).astype(BF16)
                yield

        def c2_pieces(rb):
            rows = slice(rb * TM0, (rb + 1) * TM0)
            y = None
            hs = []
            for f in range(F // 128):
                fs = slice(f * 128, (f + 1) * 128)
                g = jnp.dot(xn_s[rows, :], wg_ref[:, fs], preferred_element_type=F32)
                yield
                u = jnp.dot(xn_s[rows, :], wu_ref[:, fs], preferred_element_type=F32)
                hs.append((g * u).astype(BF16))
                yield
                if f >= 1:
                    a = jnp.dot(hs[f - 1], wd_ref[(f - 1) * 128:f * 128, :], preferred_element_type=F32)
                    y = a if y is None else a + y
                    yield
            a = jnp.dot(hs[-1], wd_ref[F - 128:F, :], preferred_element_type=F32)
            y = x_s[rows, :] + (a + y)
            x_s[rows, :] = y
            out_s[rows, :] = y.astype(BF16)
            yield

        def chain(*gens):
            for g in gens:
                yield from g

        def c2(r0):
            rows = pl.ds(r0, TMC)
            xn = xn_s[rows, :]
            g = jnp.dot(xn, wg_ref[...], preferred_element_type=F32)
            u = jnp.dot(xn, wu_ref[...], preferred_element_type=F32)
            hh = (g * u).astype(BF16)
            y = x_s[rows, :] + jnp.dot(hh, wd_ref[...], preferred_element_type=F32)
            x_s[rows, :] = y
            out_s[rows, :] = y.astype(BF16)

        def layer(li, carry):
            first = li == 0
            last = li == 1
            phase_a(first)
            def pro(_, c):
                for hh in range(8):
                    att_unit(lax.shift_right_logical(li, 1), None, hh, pattern0)
                return c
            if split_ab == 2:
                pl.when(li >= 0)(lambda: pro(0, None))
            elif split_ab == 3:
                lax.fori_loop(li, li + 1, pro, 0)

            else:
                pro(0, 0)

            if only == "pro":
                out_s[0:8, :] = s_s[0, 0:8, :].astype(BF16) + m_s[0].astype(BF16)
                return carry

            def body(b, c):
                if shift:
                    s1_tail(b, CK)
                for hh in range(8):
                    att_unit(b + 1, b, hh, pattern)
                return c
            lax.fori_loop(0, NB - 1, body, 0)

            @pl.when(first)
            def _():
                for i in range(1, 5):
                    w_copy(i).wait()

            n1 = (S - TQ) // TM0
            pieces = chain(*[c1_pieces(rb) for rb in range(n1)], c2_pieces(0))
            if shift:
                s1_tail(NB - 1, CK)
            for hh in range(8):
                att_unit(None, NB - 1, hh, pattern, pieces)
            for _ in pieces:
                pass
            for n, _ in enumerate(c2_pieces(1)):
                if n == c1pos:
                    for _ in chain(*[c1_pieces(rb) for rb in range(n1, S // TM0)]):
                        pass

            @pl.when(last)
            def _():
                o_copy(0, 0, TM0).start()
                o_copy(1, TM0, TM0).start()

            def cbody(t, c):
                npc = -(-TMA // 128 // NCL) if NCL < TMA // 128 else 1
                piece = jnp.minimum(t * npc, TMA // 128 - npc)
                prow = pl.ds(pl.multiple_of(piece * 128, 128), npc * 128)
                xa_s[prow, :] = _ln(x_s[prow, :]).astype(BF16)
                r0 = pl.multiple_of(2 * TM0 + t * TMC, TM0)
                c2(r0)

                @pl.when(last)
                def _():
                    o_copy(2 + t, r0, TMC).start()
                return c
            lax.fori_loop(0, NCL, cbody, 0)
            return carry

        lax.fori_loop(0, 2, layer, 0)
        for i, (r0, n) in enumerate(out_tiles):
            o_copy(i, r0, n).wait()

    @jax.jit
    def run(A_x, A_wqkv, A_wo, B_x, B_w_gate, B_w_up, B_w_down):
        x = A_x.reshape(S, D)
        out = pl.pallas_call(
            kernel,
            out_shape=jax.ShapeDtypeStruct((S, D), A_x.dtype),
            in_specs=[pl.BlockSpec(memory_space=pl.ANY)] * 6,
            out_specs=pl.BlockSpec(memory_space=pl.ANY),
            scratch_shapes=[
                pltpu.VMEM((S, D), BF16),
                pltpu.VMEM((D, 3 * D), BF16),
                pltpu.VMEM((D, D), BF16),
                pltpu.VMEM((D, F), BF16),
                pltpu.VMEM((D, F), BF16),
                pltpu.VMEM((F, D), BF16),
                pltpu.VMEM((S, D), BF16),
                pltpu.VMEM((S, D), F32),
                pltpu.VMEM((TMA, D), BF16),
                pltpu.VMEM((S, D), BF16),
                pltpu.VMEM((2 * D, D), BF16),
                pltpu.VMEM((NROT, 4, S // 2, 128), jnp.uint32) if ku32 else pltpu.VMEM((NROT, 4, S, 128), BF16),
                pltpu.VMEM((4, S, 128), F32),
                pltpu.VMEM((D, S), BF16),
                pltpu.VMEM((S // 128, D, 8, 128), F32),
                pltpu.VMEM((D, S), F32),
                pltpu.VMEM((D, S), BF16),
                pltpu.VMEM((8, S, TQ), F32),
                pltpu.VMEM((8, 1, TQ), F32),
                pltpu.VMEM((8, TQ), F32),
                pltpu.SemaphoreType.DMA((2,)),
                pltpu.SemaphoreType.DMA((5,)),
                pltpu.SemaphoreType.DMA((len(out_tiles),)),
            ],
            compiler_params=pltpu.CompilerParams(vmem_limit_bytes=124 * 1024 * 1024),
        )(x, A_wqkv, A_wo, B_w_gate, B_w_up, B_w_down)
        return out.reshape(1, S, D)
    return run


_run = make()


def pallas_interleave_layers__softmax_full_mha__glu_gated_bilinear__prompt_kernel(
    A_x, A_wqkv, A_wo, B_x, B_w_gate, B_w_up, B_w_down
):
    return _run(A_x, A_wqkv, A_wo, B_x, B_w_gate, B_w_up, B_w_down)
```

```python
import math

import jax
import jax.numpy as jnp
from jax import lax
import jax.experimental.pallas as pl
import jax.experimental.pallas.tpu as pltpu

S, D, H, DH, F = 2048, 512, 32, 16, 1792
EPS = 1e-5
BF16 = jnp.bfloat16
F32 = jnp.float32
TQ = 512
CK = 128
NC = S // CK
NB = (H // 8) * (S // TQ)
NA = S // TQ
TM = 256
NCT = S // TM
NROT = 4
HPR = 8 // NROT
VMAX = 32
QSCALE = (DH ** -0.5) * math.log2(math.e)


def _ln(x):
    m = jnp.mean(x, axis=-1, keepdims=True)
    xc = x - m
    v = jnp.mean(xc * xc, axis=-1, keepdims=True)
    return xc * lax.rsqrt(v + EPS)


def _mo(v, m):
    return v if isinstance(v, int) else pl.multiple_of(v, m)


def _chain(*gens):
    for g in gens:
        yield from g


def make(pattern="1111111111110000", pattern0="2111211121112110", npx=96, c1pos=2, interp=False):

    def kernel(x_hbm, wqkv_hbm, wo_hbm, wg_hbm, wu_hbm, wd_hbm, o_hbm,
               xin_s, wqkv_ref, wo_ref, wg_ref, wu_ref, wd_ref, out_s,
               x_s, xa_s, xn_s, wqvT_s, k_s, kf_s, qT_s, qb_s, vT_s, oT_s, s_s, m_s,
               sem_x, sem_w, sem_o):
        def x_copy(t):
            rows = slice(t * TQ, (t + 1) * TQ) if t < 2 else slice(2 * TQ, S)
            return pltpu.make_async_copy(x_hbm.at[rows, :], xin_s.at[rows, :], sem_x.at[t])

        def wqkv_copy(i):
            cols = slice(i * D, (i + 1) * D)
            return pltpu.make_async_copy(wqkv_hbm.at[:, cols], wqkv_ref.at[:, cols], sem_x.at[3 + i])

        w_pairs = ((wo_hbm, wo_ref), (wg_hbm, wg_ref), (wu_hbm, wu_ref), (wd_hbm, wd_ref))

        def w_copy(i):
            return pltpu.make_async_copy(w_pairs[i][0], w_pairs[i][1], sem_w.at[i])

        def o_copy(t):
            rows = pl.ds(_mo(t * TM, TM), TM)
            return pltpu.make_async_copy(out_s.at[rows, :], o_hbm.at[rows, :], sem_o.at[t])

        x_copy(0).start()
        wqkv_copy(1).start()
        x_copy(0).wait()
        wqkv_copy(0).start()
        wqkv_copy(2).start()
        xa_s[...] = _ln(xin_s[0:TQ, :].astype(F32)).astype(BF16)
        wqkv_copy(1).wait()
        x_copy(1).start()
        x_copy(2).start()

        def x_in(first, rows):
            return jnp.where(first, xin_s[rows, :].astype(F32), x_s[rows, :])

        def transpose_weights():
            wqT = wqkv_ref[:, 0:D].astype(F32).T.astype(BF16)
            wvT = wqkv_ref[:, 2 * D:3 * D].astype(F32).T.astype(BF16)
            for h in range(H):
                wqvT_s[2 * h * DH:(2 * h + 1) * DH, :] = wqT[h * DH:(h + 1) * DH]
                wqvT_s[(2 * h + 1) * DH:(2 * h + 2) * DH, :] = wvT[h * DH:(h + 1) * DH]

        def proj_k(t, xn):
            kk = jnp.dot(xn, wqkv_ref[:, D:2 * D], preferred_element_type=F32)
            for g in range(4):
                kg = kk[:, g * 128:(g + 1) * 128]
                for i in range(TQ // CK):
                    kf_s[g, t * (TQ // CK) + i] = kg[(i + 1) * CK - VMAX:(i + 1) * CK]
                for r in range(NROT):
                    kb16 = (kg if r == 0 else pltpu.roll(kg, 128 - r * HPR * DH, 1)).astype(BF16)
                    k_s[r, g, t * TQ // 2:(t + 1) * TQ // 2, :] = pltpu.bitcast(kb16, jnp.uint32)

        def proj_qv(t, xn):
            cols = slice(t * TQ, (t + 1) * TQ)
            qv = lax.dot_general(wqvT_s[...], xn, (((1,), (1,)), ((), ())), preferred_element_type=F32)
            qv = qv.reshape(H, 2 * DH, TQ)
            q = qv[:, 0:DH, :].reshape(D, TQ) * QSCALE
            qT_s[:, cols] = q.astype(BF16)
            for c in range(TQ // 128):
                qc = q[:, c * 128:(c + 1) * 128]
                qb_s[t, :, :, c * 128:(c + 1) * 128] = jnp.broadcast_to(qc[:, None, :], (D, 8, 128))
            vT_s[:, cols] = qv[:, DH:2 * DH, :].reshape(D, TQ)

        def phase_a(first, always):
            def ln_tile(t):
                rows = slice(t * TQ, (t + 1) * TQ)
                xn_s[rows, :] = _ln(x_in(first, rows)).astype(BF16)

            def xn(t):
                return xn_s[t * TQ:(t + 1) * TQ, :]

            proj_k(0, xa_s[...])

            @pl.when(first)
            def _():
                wqkv_copy(0).wait()
                wqkv_copy(2).wait()
                transpose_weights()
                x_copy(1).wait()

            ln_tile(1)
            proj_qv(0, xa_s[...])

            @pl.when(first)
            def _():
                x_copy(2).wait()
                for i in range(4):
                    w_copy(i).start()

            ln_tile(2)
            proj_k(1, xn(1))
            proj_qv(1, xn(1))
            ln_tile(3)
            proj_k(2, xn(2))
            proj_qv(2, xn(2))

            @pl.when(always)
            def _():
                proj_k(3, xn(3))
                proj_qv(3, xn(3))

        def att_unit(b1, b2, hh, pat, pieces=None):
            vr = [16 * int(ch) for ch in pat]
            items = [(i, r) for i in range(NC) for r in range(VMAX - vr[i], VMAX, 8)]
            l8 = None
            acc = None
            m8 = None
            if b2 is not None:
                g2, j2 = b2 % 4, b2 // 4
                mb = jnp.broadcast_to(m_s[hh], (8, TQ))
                hrows = pl.ds(_mo((g2 * 8 + hh) * DH, DH), DH)
            if b1 is not None:
                g1, j1 = b1 % 4, b1 // 4
                hp = hh % HPR
                qrows = pl.ds(_mo((g1 * 8 + hh) * DH, DH), DH)
                parts = [qT_s[qrows, pl.ds(_mo(j1 * TQ, TQ), TQ)], jnp.zeros((DH * (7 - hp), TQ), BF16)]
                if hp > 0:
                    parts.insert(0, jnp.zeros((DH * hp, TQ), BF16))
                qm = jnp.concatenate(parts, axis=0)
                onehot = (lax.broadcasted_iota(jnp.int32, (DH, 8, 128), 2)
                          == lax.broadcasted_iota(jnp.int32, (DH, 8, 128), 0) + hh * DH)

            def v_item(idx):
                i, r = items[idx]
                zz = lax.shift_right_logical(b1, 5 + idx % 26)
                kf = kf_s[pl.ds(g1 + zz, 1), i, r:r + 8, :]
                kb = jnp.sum(jnp.where(onehot, kf, 0.0), axis=2, keepdims=True)
                qd = qb_s[pl.ds(j1 + zz, 1), qrows][0]
                sv = jnp.sum(kb * qd, axis=0)
                r0 = (i + 1) * CK - VMAX + r
                s_s[hh, r0:r0 + 8, :] = sv
                return sv

            tot_rg = (S - sum(vr)) // 8
            rg_done = 0
            vdone = 0
            for i in range(NC):
                sl = slice(i * CK, (i + 1) * CK)
                n = hh * NC + i
                if pieces is not None and n * npx // (8 * NC) != (n + 1) * npx // (8 * NC):
                    next(pieces)
                if b2 is not None:
                    sp = s_s[hh, sl, :].reshape(CK // 8, 8, TQ)
                    p = jnp.exp2(sp - mb[None]).reshape(CK, TQ)
                    for r in range(CK // 8 - 1, -1, -1):
                        pr = p[r * 8:(r + 1) * 8, :]
                        l8 = pr if l8 is None else l8 + pr
                    a = jnp.dot(vT_s[hrows, sl], p, preferred_element_type=F32)
                    acc = a if acc is None else a + acc
                if b1 is not None:
                    lo, hi = i * CK, (i + 1) * CK - vr[i]
                    kr = pltpu.bitcast(k_s[hh // HPR, pl.ds(g1, 1), lo // 2:hi // 2, :][0], BF16)
                    sT = jnp.dot(kr, qm, preferred_element_type=F32)
                    s_s[hh, lo:hi, :] = sT
                    for r in range((hi - lo) // 8):
                        sr = sT[r * 8:(r + 1) * 8, :]
                        m8 = sr if m8 is None else jnp.maximum(m8, sr)
                        rg_done += 1
                        want = rg_done * len(items) // tot_rg
                        while vdone < want and (b2 is None or items[vdone][0] <= i):
                            m8 = jnp.maximum(m8, v_item(vdone))
                            vdone += 1
            if b2 is not None:
                l = jnp.sum(l8, axis=0, keepdims=True)
                oT_s[hrows, pl.ds(_mo(j2 * TQ, TQ), TQ)] = (acc * (1.0 / l)).astype(BF16)
            if b1 is not None:
                assert vdone == len(items)
                m_s[hh] = jnp.max(m8, axis=0, keepdims=True)

        def c1_pieces(rb, first):
            rows = slice(rb * TM, (rb + 1) * TM)
            o = oT_s[:, rows].T
            cols = []
            for c in range(D // 128):
                cols.append(jnp.dot(o, wo_ref[:, c * 128:(c + 1) * 128], preferred_element_type=F32))
                if c == D // 128 - 1:
                    x1 = x_in(first, rows) + jnp.concatenate(cols, axis=1)
                    x_s[rows, :] = x1
                    xn_s[rows, :] = _ln(x1).astype(BF16)
                yield

        def c2_pieces(rb):
            rows = slice(rb * TM, (rb + 1) * TM)
            y = None
            hs = []
            for f in range(F // 128):
                fs = slice(f * 128, (f + 1) * 128)
                g = jnp.dot(xn_s[rows, :], wg_ref[:, fs], preferred_element_type=F32)
                yield
                u = jnp.dot(xn_s[rows, :], wu_ref[:, fs], preferred_element_type=F32)
                hs.append((g * u).astype(BF16))
                yield
                if f >= 1:
                    a = jnp.dot(hs[f - 1], wd_ref[(f - 1) * 128:f * 128, :], preferred_element_type=F32)
                    y = a if y is None else a + y
                    yield
            a = jnp.dot(hs[-1], wd_ref[F - 128:F, :], preferred_element_type=F32)
            y = x_s[rows, :] + (a + y)
            x_s[rows, :] = y
            out_s[rows, :] = y.astype(BF16)
            yield

        def c2(t):
            rows = pl.ds(_mo(t * TM, TM), TM)
            xn = xn_s[rows, :]
            g = jnp.dot(xn, wg_ref[...], preferred_element_type=F32)
            u = jnp.dot(xn, wu_ref[...], preferred_element_type=F32)
            hh = (g * u).astype(BF16)
            y = x_s[rows, :] + jnp.dot(hh, wd_ref[...], preferred_element_type=F32)
            x_s[rows, :] = y
            out_s[rows, :] = y.astype(BF16)

        def layer(li, carry):
            first = li == 0
            last = li == 1
            phase_a(first, li < 2)

            @pl.when(li >= 0)
            def _():
                for hh in range(8):
                    att_unit(lax.shift_right_logical(li, 1), None, hh, pattern0)

            def body(b, c):
                for hh in range(8):
                    att_unit(b + 1, b, hh, pattern)
                return c
            lax.fori_loop(0, NB - 1, body, 0)

            @pl.when(first)
            def _():
                for i in range(4):
                    w_copy(i).wait()

            n1 = (S - TQ) // TM
            pieces = _chain(*[c1_pieces(rb, first) for rb in range(n1)], c2_pieces(0), c2_pieces(1))
            for hh in range(8):
                att_unit(None, NB - 1, hh, pattern, pieces)
            for n, _ in enumerate(pieces):
                if n == c1pos:
                    for _ in _chain(*[c1_pieces(rb, first) for rb in range(n1, NCT)]):
                        pass

            @pl.when(last)
            def _():
                o_copy(0).start()
                o_copy(1).start()

            def cbody(t, c):
                piece = jnp.minimum(t - 2, TQ // 128 - 1)
                prow = pl.ds(pl.multiple_of(piece * 128, 128), 128)
                xa_s[prow, :] = _ln(x_s[prow, :]).astype(BF16)
                c2(t)

                @pl.when(last)
                def _():
                    o_copy(t).start()
                return c
            lax.fori_loop(2, NCT, cbody, 0)
            return carry

        lax.fori_loop(0, 2, layer, 0)
        for t in range(NCT):
            o_copy(t).wait()

    @jax.jit
    def run(A_x, A_wqkv, A_wo, B_x, B_w_gate, B_w_up, B_w_down):
        x = A_x.reshape(S, D)
        out = pl.pallas_call(
            kernel,
            out_shape=jax.ShapeDtypeStruct((S, D), A_x.dtype),
            in_specs=[pl.BlockSpec(memory_space=pl.ANY)] * 6,
            out_specs=pl.BlockSpec(memory_space=pl.ANY),
            scratch_shapes=[
                pltpu.VMEM((S, D), BF16),
                pltpu.VMEM((D, 3 * D), BF16),
                pltpu.VMEM((D, D), BF16),
                pltpu.VMEM((D, F), BF16),
                pltpu.VMEM((D, F), BF16),
                pltpu.VMEM((F, D), BF16),
                pltpu.VMEM((S, D), BF16),
                pltpu.VMEM((S, D), F32),
                pltpu.VMEM((TQ, D), BF16),
                pltpu.VMEM((S, D), BF16),
                pltpu.VMEM((2 * D, D), BF16),
                pltpu.VMEM((NROT, 4, S // 2, 128), jnp.uint32),
                pltpu.VMEM((4, NC, VMAX, 128), F32),
                pltpu.VMEM((D, S), BF16),
                pltpu.VMEM((NA, D, 8, TQ), F32),
                pltpu.VMEM((D, S), F32),
                pltpu.VMEM((D, S), BF16),
                pltpu.VMEM((8, S, TQ), F32),
                pltpu.VMEM((8, 1, TQ), F32),
                pltpu.SemaphoreType.DMA((6,)),
                pltpu.SemaphoreType.DMA((4,)),
                pltpu.SemaphoreType.DMA((NCT,)),
            ],
            compiler_params=pltpu.CompilerParams(vmem_limit_bytes=120 * 1024 * 1024),
            interpret=interp,
        )(x, A_wqkv, A_wo, B_w_gate, B_w_up, B_w_down)
        return out.reshape(1, S, D)
    return run


_run = make()


def pallas_interleave_layers__softmax_full_mha__glu_gated_bilinear__prompt_kernel(
    A_x, A_wqkv, A_wo, B_x, B_w_gate, B_w_up, B_w_down
):
    return _run(A_x, A_wqkv, A_wo, B_x, B_w_gate, B_w_up, B_w_down)
```

```python
import math

import jax
import jax.numpy as jnp
from jax import lax
import jax.experimental.pallas as pl
import jax.experimental.pallas.tpu as pltpu

S, D, H, DH, F = 2048, 512, 32, 16, 1792
EPS = 1e-5
BF16 = jnp.bfloat16
F32 = jnp.float32
TQ = 512
CK = 128
NC = S // CK
NB = (H // 8) * (S // TQ)
NA = S // TQ
TM = 256
NCT = S // TM
NROT = 4
HPR = 8 // NROT
VMAX = 32
QSCALE = (DH ** -0.5) * math.log2(math.e)


def _ln(x):
    m = jnp.mean(x, axis=-1, keepdims=True)
    xc = x - m
    v = jnp.mean(xc * xc, axis=-1, keepdims=True)
    return xc * lax.rsqrt(v + EPS)


def _mo(v, m):
    return v if isinstance(v, int) else pl.multiple_of(v, m)


def _chain(*gens):
    for g in gens:
        yield from g


def make(npx=96, c1pos=2, interp=False):
    pattern = "1111111111110000"
    pattern_first = "2111111111110000"
    pattern_last = "1111111111111000"
    pattern0 = "2111211121112110"

    def kernel(x_hbm, wqkv_hbm, wo_hbm, wg_hbm, wu_hbm, wd_hbm, o_hbm,
               xin_s, wqkv_ref, wo_ref, wg_ref, wu_ref, wd_ref, out_s,
               x_s, xa_s, xn_s, wqvT_s, k_s, kf_s, qT_s, qb_s, vT_s, oT_s, s_s, m_s,
               sem_x, sem_w, sem_o):
        def x_copy(t):
            rows = slice(t * TQ, (t + 1) * TQ) if t < 2 else slice(2 * TQ, S)
            return pltpu.make_async_copy(x_hbm.at[rows, :], xin_s.at[rows, :], sem_x.at[t])

        def wqkv_copy(i):
            cols = slice(i * D, (i + 1) * D)
            return pltpu.make_async_copy(wqkv_hbm.at[:, cols], wqkv_ref.at[:, cols], sem_x.at[3 + i])

        w_pairs = ((wo_hbm, wo_ref), (wg_hbm, wg_ref), (wu_hbm, wu_ref), (wd_hbm, wd_ref))

        def w_copy(i):
            return pltpu.make_async_copy(w_pairs[i][0], w_pairs[i][1], sem_w.at[i])

        def o_copy(t):
            rows = pl.ds(_mo(t * TM, TM), TM)
            return pltpu.make_async_copy(out_s.at[rows, :], o_hbm.at[rows, :], sem_o.at[t])

        x_copy(0).start()
        wqkv_copy(1).start()
        x_copy(0).wait()
        wqkv_copy(0).start()
        wqkv_copy(2).start()
        xa_s[...] = _ln(xin_s[0:TQ, :].astype(F32)).astype(BF16)
        wqkv_copy(1).wait()
        x_copy(1).start()
        x_copy(2).start()

        def x_in(first, rows):
            return jnp.where(first, xin_s[rows, :].astype(F32), x_s[rows, :])

        def transpose_weights():
            wqT = wqkv_ref[:, 0:D].astype(F32).T.astype(BF16)
            wvT = wqkv_ref[:, 2 * D:3 * D].astype(F32).T.astype(BF16)
            for h in range(H):
                wqvT_s[2 * h * DH:(2 * h + 1) * DH, :] = wqT[h * DH:(h + 1) * DH]
                wqvT_s[(2 * h + 1) * DH:(2 * h + 2) * DH, :] = wvT[h * DH:(h + 1) * DH]

        def proj_k(t, xn):
            kk = jnp.dot(xn, wqkv_ref[:, D:2 * D], preferred_element_type=F32)
            for g in range(4):
                kg = kk[:, g * 128:(g + 1) * 128]
                for i in range(TQ // CK):
                    kf_s[g, t * (TQ // CK) + i] = kg[(i + 1) * CK - VMAX:(i + 1) * CK]
                for r in range(NROT):
                    kb16 = (kg if r == 0 else pltpu.roll(kg, 128 - r * HPR * DH, 1)).astype(BF16)
                    k_s[r, g, t * TQ // 2:(t + 1) * TQ // 2, :] = pltpu.bitcast(kb16, jnp.uint32)

        def proj_qv(t, xn):
            cols = slice(t * TQ, (t + 1) * TQ)
            qv = lax.dot_general(wqvT_s[...], xn, (((1,), (1,)), ((), ())), preferred_element_type=F32)
            qv = qv.reshape(H, 2 * DH, TQ)
            q = qv[:, 0:DH, :].reshape(D, TQ) * QSCALE
            qT_s[:, cols] = q.astype(BF16)
            for c in range(TQ // 128):
                qc = q[:, c * 128:(c + 1) * 128]
                qb_s[t, :, :, c * 128:(c + 1) * 128] = jnp.broadcast_to(qc[:, None, :], (D, 8, 128))
            vT_s[:, cols] = qv[:, DH:2 * DH, :].reshape(D, TQ)

        def phase_a(first, always):
            def ln_tile(t):
                rows = slice(t * TQ, (t + 1) * TQ)
                xn_s[rows, :] = _ln(x_in(first, rows)).astype(BF16)

            def xn(t):
                return xn_s[t * TQ:(t + 1) * TQ, :]

            proj_k(0, xa_s[...])

            @pl.when(first)
            def _():
                wqkv_copy(0).wait()
                wqkv_copy(2).wait()
                transpose_weights()
                x_copy(1).wait()

            ln_tile(1)
            proj_qv(0, xa_s[...])

            @pl.when(first)
            def _():
                x_copy(2).wait()
                for i in range(4):
                    w_copy(i).start()

            ln_tile(2)
            proj_k(1, xn(1))
            proj_qv(1, xn(1))
            ln_tile(3)
            proj_k(2, xn(2))
            proj_qv(2, xn(2))

            @pl.when(always)
            def _():
                proj_k(3, xn(3))
                proj_qv(3, xn(3))

        def att_unit(b1, b2, hh, pat, pieces=None, nf=0, nl=0):
            vr = [16 * int(ch) for ch in pat]
            items = [(i, r) for i in range(NC) for r in range(VMAX - vr[i], VMAX, 8)]
            l8 = None
            acc = None
            m8 = None
            if b2 is not None:
                g2, j2 = b2 % 4, b2 // 4
                mb = jnp.broadcast_to(m_s[hh], (8, TQ))
                hrows = pl.ds(_mo((g2 * 8 + hh) * DH, DH), DH)
            if b1 is not None:
                g1, j1 = b1 % 4, b1 // 4
                hp = hh % HPR
                qrows = pl.ds(_mo((g1 * 8 + hh) * DH, DH), DH)
                parts = [qT_s[qrows, pl.ds(_mo(j1 * TQ, TQ), TQ)], jnp.zeros((DH * (7 - hp), TQ), BF16)]
                if hp > 0:
                    parts.insert(0, jnp.zeros((DH * hp, TQ), BF16))
                qm = jnp.concatenate(parts, axis=0)
                onehot = (lax.broadcasted_iota(jnp.int32, (DH, 8, 128), 2)
                          == lax.broadcasted_iota(jnp.int32, (DH, 8, 128), 0) + hh * DH)

            def v_item(idx):
                i, r = items[idx]
                zz = lax.shift_right_logical(b1, 5 + idx % 26)
                kf = kf_s[pl.ds(g1 + zz, 1), i, r:r + 8, :]
                kb = jnp.sum(jnp.where(onehot, kf, 0.0), axis=2, keepdims=True)
                qd = qb_s[pl.ds(j1 + zz, 1), qrows][0]
                sv = jnp.sum(kb * qd, axis=0)
                r0 = (i + 1) * CK - VMAX + r
                s_s[hh, r0:r0 + 8, :] = sv
                return sv

            tot_rg = (S - sum(vr)) // 8
            rg_done = 0
            vdone = 0
            for i in range(NC):
                sl = slice(i * CK, (i + 1) * CK)
                n = hh * NC + i
                if pieces is not None and n * npx // (8 * NC) != (n + 1) * npx // (8 * NC):
                    next(pieces)
                if b2 is not None:
                    sp = s_s[hh, sl, :].reshape(CK // 8, 8, TQ)
                    p = jnp.exp2(sp - mb[None]).reshape(CK, TQ)
                    for r in range(CK // 8 - 1, -1, -1):
                        pr = p[r * 8:(r + 1) * 8, :]
                        l8 = pr if l8 is None else l8 + pr
                    a = jnp.dot(vT_s[hrows, sl], p, preferred_element_type=F32)
                    acc = a if acc is None else a + acc
                if b1 is not None:
                    lo, hi = i * CK, (i + 1) * CK - vr[i]
                    kr = pltpu.bitcast(k_s[hh // HPR, pl.ds(g1, 1), lo // 2:hi // 2, :][0], BF16)
                    sT = jnp.dot(kr, qm, preferred_element_type=F32)
                    s_s[hh, lo:hi, :] = sT
                    for r in range((hi - lo) // 8):
                        sr = sT[r * 8:(r + 1) * 8, :]
                        m8 = sr if m8 is None else jnp.maximum(m8, sr)
                        rg_done += 1
                        want = nf + rg_done * (len(items) - nf - nl) // tot_rg + (nl if rg_done == tot_rg else 0)
                        while vdone < want and (b2 is None or items[vdone][0] <= i):
                            m8 = jnp.maximum(m8, v_item(vdone))
                            vdone += 1
            if b2 is not None:
                l = jnp.sum(l8, axis=0, keepdims=True)
                oT_s[hrows, pl.ds(_mo(j2 * TQ, TQ), TQ)] = (acc * (1.0 / l)).astype(BF16)
            if b1 is not None:
                assert vdone == len(items)
                m_s[hh] = jnp.max(m8, axis=0, keepdims=True)

        def c1_pieces(rb, first):
            rows = slice(rb * TM, (rb + 1) * TM)
            o = oT_s[:, rows].T
            cols = []
            for c in range(D // 128):
                cols.append(jnp.dot(o, wo_ref[:, c * 128:(c + 1) * 128], preferred_element_type=F32))
                if c == D // 128 - 1:
                    x1 = x_in(first, rows) + jnp.concatenate(cols, axis=1)
                    x_s[rows, :] = x1
                    xn_s[rows, :] = _ln(x1).astype(BF16)
                yield

        def c2_pieces(rb):
            rows = slice(rb * TM, (rb + 1) * TM)
            y = None
            hs = []
            for f in range(F // 128):
                fs = slice(f * 128, (f + 1) * 128)
                g = jnp.dot(xn_s[rows, :], wg_ref[:, fs], preferred_element_type=F32)
                yield
                u = jnp.dot(xn_s[rows, :], wu_ref[:, fs], preferred_element_type=F32)
                hs.append((g * u).astype(BF16))
                yield
                if f >= 1:
                    a = jnp.dot(hs[f - 1], wd_ref[(f - 1) * 128:f * 128, :], preferred_element_type=F32)
                    y = a if y is None else a + y
                    yield
            a = jnp.dot(hs[-1], wd_ref[F - 128:F, :], preferred_element_type=F32)
            y = x_s[rows, :] + (a + y)
            x_s[rows, :] = y
            out_s[rows, :] = y.astype(BF16)
            yield

        def c2(t):
            rows = pl.ds(_mo(t * TM, TM), TM)
            xn = xn_s[rows, :]
            g = jnp.dot(xn, wg_ref[...], preferred_element_type=F32)
            u = jnp.dot(xn, wu_ref[...], preferred_element_type=F32)
            hh = (g * u).astype(BF16)
            y = x_s[rows, :] + jnp.dot(hh, wd_ref[...], preferred_element_type=F32)
            x_s[rows, :] = y
            out_s[rows, :] = y.astype(BF16)

        def layer(li, carry):
            first = li == 0
            last = li == 1
            phase_a(first, li < 2)

            @pl.when(li >= 0)
            def _():
                for hh in range(8):
                    att_unit(lax.shift_right_logical(li, 1), None, hh, pattern0)

            def body(b, c):
                att_unit(b + 1, b, 0, pattern_first, nf=2)
                for hh in range(1, 7):
                    att_unit(b + 1, b, hh, pattern)
                att_unit(b + 1, b, 7, pattern_last, nl=2)
                return c
            lax.fori_loop(0, NB - 1, body, 0)

            @pl.when(first)
            def _():
                for i in range(4):
                    w_copy(i).wait()

            n1 = (S - TQ) // TM
            pieces = _chain(*[c1_pieces(rb, first) for rb in range(n1)], c2_pieces(0), c2_pieces(1))
            for hh in range(8):
                att_unit(None, NB - 1, hh, pattern, pieces)
            for n, _ in enumerate(pieces):
                if n == c1pos:
                    for _ in _chain(*[c1_pieces(rb, first) for rb in range(n1, NCT)]):
                        pass

            @pl.when(last)
            def _():
                o_copy(0).start()
                o_copy(1).start()

            def cbody(t, c):
                piece = jnp.minimum(t - 2, TQ // 128 - 1)
                prow = pl.ds(pl.multiple_of(piece * 128, 128), 128)
                xa_s[prow, :] = _ln(x_s[prow, :]).astype(BF16)
                c2(t)

                @pl.when(last)
                def _():
                    o_copy(t).start()
                return c
            lax.fori_loop(2, NCT, cbody, 0)
            return carry

        lax.fori_loop(0, 2, layer, 0)
        for t in range(NCT):
            o_copy(t).wait()

    @jax.jit
    def run(A_x, A_wqkv, A_wo, B_x, B_w_gate, B_w_up, B_w_down):
        x = A_x.reshape(S, D)
        out = pl.pallas_call(
            kernel,
            out_shape=jax.ShapeDtypeStruct((S, D), A_x.dtype),
            in_specs=[pl.BlockSpec(memory_space=pl.ANY)] * 6,
            out_specs=pl.BlockSpec(memory_space=pl.ANY),
            scratch_shapes=[
                pltpu.VMEM((S, D), BF16),
                pltpu.VMEM((D, 3 * D), BF16),
                pltpu.VMEM((D, D), BF16),
                pltpu.VMEM((D, F), BF16),
                pltpu.VMEM((D, F), BF16),
                pltpu.VMEM((F, D), BF16),
                pltpu.VMEM((S, D), BF16),
                pltpu.VMEM((S, D), F32),
                pltpu.VMEM((TQ, D), BF16),
                pltpu.VMEM((S, D), BF16),
                pltpu.VMEM((2 * D, D), BF16),
                pltpu.VMEM((NROT, 4, S // 2, 128), jnp.uint32),
                pltpu.VMEM((4, NC, VMAX, 128), F32),
                pltpu.VMEM((D, S), BF16),
                pltpu.VMEM((NA, D, 8, TQ), F32),
                pltpu.VMEM((D, S), F32),
                pltpu.VMEM((D, S), BF16),
                pltpu.VMEM((8, S, TQ), F32),
                pltpu.VMEM((8, 1, TQ), F32),
                pltpu.SemaphoreType.DMA((6,)),
                pltpu.SemaphoreType.DMA((4,)),
                pltpu.SemaphoreType.DMA((NCT,)),
            ],
            compiler_params=pltpu.CompilerParams(vmem_limit_bytes=120 * 1024 * 1024),
            interpret=interp,
        )(x, A_wqkv, A_wo, B_w_gate, B_w_up, B_w_down)
        return out.reshape(1, S, D)
    return run


_run = make()


def pallas_interleave_layers__softmax_full_mha__glu_gated_bilinear__prompt_kernel(
    A_x, A_wqkv, A_wo, B_x, B_w_gate, B_w_up, B_w_down
):
    return _run(A_x, A_wqkv, A_wo, B_x, B_w_gate, B_w_up, B_w_down)
```

```python
import math

import jax
import jax.numpy as jnp
from jax import lax
import jax.experimental.pallas as pl
import jax.experimental.pallas.tpu as pltpu

S, D, H, DH, F = 2048, 512, 32, 16, 1792
EPS = 1e-5
BF16 = jnp.bfloat16
F32 = jnp.float32
TQ = 512
CK = 128
NC = S // CK
NB = (H // 8) * (S // TQ)
NA = S // TQ
TM = 256
NCT = S // TM
NROT = 4
HPR = 8 // NROT
VMAX = 32
QSCALE = (DH ** -0.5) * math.log2(math.e)


def _ln(x):
    m = jnp.mean(x, axis=-1, keepdims=True)
    xc = x - m
    v = jnp.mean(xc * xc, axis=-1, keepdims=True)
    return xc * lax.rsqrt(v + EPS)


def _mo(v, m):
    return v if isinstance(v, int) else pl.multiple_of(v, m)


def _chain(*gens):
    for g in gens:
        yield from g


def _make():
    npx = 96
    c1pos = 2
    pattern = "1111111111110000"
    pattern_first = "2111111111110000"
    pattern_last = "1111111111111000"
    pattern0 = "2111211121112110"

    def kernel(x_hbm, wqkv_hbm, wo_hbm, wg_hbm, wu_hbm, wd_hbm, o_hbm,
               xin_s, wqkv_ref, wo_ref, wg_ref, wu_ref, wd_ref, out_s,
               x_s, xa_s, xn_s, wqvT_s, k_s, kf_s, qT_s, qb_s, vT_s, oT_s, s_s, m_s,
               sem_x, sem_w, sem_o):
        def x_copy(t):
            rows = slice(t * TQ, (t + 1) * TQ) if t < 2 else slice(2 * TQ, S)
            return pltpu.make_async_copy(x_hbm.at[rows, :], xin_s.at[rows, :], sem_x.at[t])

        def wqkv_copy(i):
            cols = slice(i * D, (i + 1) * D)
            return pltpu.make_async_copy(wqkv_hbm.at[:, cols], wqkv_ref.at[:, cols], sem_x.at[3 + i])

        w_pairs = ((wo_hbm, wo_ref), (wg_hbm, wg_ref), (wu_hbm, wu_ref), (wd_hbm, wd_ref))

        def w_copy(i):
            return pltpu.make_async_copy(w_pairs[i][0], w_pairs[i][1], sem_w.at[i])

        def o_copy(t):
            rows = pl.ds(_mo(t * TM, TM), TM)
            return pltpu.make_async_copy(out_s.at[rows, :], o_hbm.at[rows, :], sem_o.at[t])

        x_copy(0).start()
        wqkv_copy(1).start()
        x_copy(0).wait()
        wqkv_copy(0).start()
        wqkv_copy(2).start()
        xa_s[...] = _ln(xin_s[0:TQ, :].astype(F32)).astype(BF16)
        wqkv_copy(1).wait()
        x_copy(1).start()
        x_copy(2).start()

        def x_in(first, rows):
            return jnp.where(first, xin_s[rows, :].astype(F32), x_s[rows, :])

        def transpose_weights():
            wqT = wqkv_ref[:, 0:D].astype(F32).T.astype(BF16)
            wvT = wqkv_ref[:, 2 * D:3 * D].astype(F32).T.astype(BF16)
            for h in range(H):
                wqvT_s[2 * h * DH:(2 * h + 1) * DH, :] = wqT[h * DH:(h + 1) * DH]
                wqvT_s[(2 * h + 1) * DH:(2 * h + 2) * DH, :] = wvT[h * DH:(h + 1) * DH]

        def proj_k(t, xn):
            kk = jnp.dot(xn, wqkv_ref[:, D:2 * D], preferred_element_type=F32)
            for g in range(4):
                kg = kk[:, g * 128:(g + 1) * 128]
                for i in range(TQ // CK):
                    kf_s[g, t * (TQ // CK) + i] = kg[(i + 1) * CK - VMAX:(i + 1) * CK]
                ku = pltpu.bitcast(kg.astype(BF16), jnp.uint32)
                for r in range(NROT):
                    k_s[r, g, t * TQ // 2:(t + 1) * TQ // 2, :] = (
                        ku if r == 0 else pltpu.roll(ku, 128 - r * HPR * DH, 1))

        def proj_qv(t, xn):
            cols = slice(t * TQ, (t + 1) * TQ)
            qv = lax.dot_general(wqvT_s[...], xn, (((1,), (1,)), ((), ())), preferred_element_type=F32)
            qv = qv.reshape(H, 2 * DH, TQ)
            q = qv[:, 0:DH, :].reshape(D, TQ) * QSCALE
            qT_s[:, cols] = q.astype(BF16)
            for c in range(TQ // 128):
                qc = q[:, c * 128:(c + 1) * 128]
                qb_s[t, :, :, c * 128:(c + 1) * 128] = jnp.broadcast_to(qc[:, None, :], (D, 8, 128))
            vT_s[:, cols] = qv[:, DH:2 * DH, :].reshape(D, TQ)

        def phase_a(first, always):
            def ln_tile(t):
                rows = slice(t * TQ, (t + 1) * TQ)
                xn_s[rows, :] = _ln(x_in(first, rows)).astype(BF16)

            def xn(t):
                return xn_s[t * TQ:(t + 1) * TQ, :]

            proj_k(0, xa_s[...])

            @pl.when(first)
            def _():
                wqkv_copy(0).wait()
                wqkv_copy(2).wait()
                transpose_weights()
                x_copy(1).wait()

            ln_tile(1)
            proj_qv(0, xa_s[...])

            @pl.when(first)
            def _():
                x_copy(2).wait()
                for i in range(4):
                    w_copy(i).start()

            ln_tile(2)
            proj_k(1, xn(1))
            proj_qv(1, xn(1))
            ln_tile(3)
            proj_k(2, xn(2))
            proj_qv(2, xn(2))

            @pl.when(always)
            def _():
                proj_k(3, xn(3))
                proj_qv(3, xn(3))

        def att_unit(b1, b2, hh, pat, pieces=None, nf=0, nl=0):
            vr = [16 * int(ch) for ch in pat]
            items = [(i, r) for i in range(NC) for r in range(VMAX - vr[i], VMAX, 8)]
            l8 = None
            acc = None
            m8 = None
            if b2 is not None:
                g2, j2 = b2 % 4, b2 // 4
                mb = jnp.broadcast_to(m_s[hh], (8, TQ))
                hrows = pl.ds(_mo((g2 * 8 + hh) * DH, DH), DH)
            if b1 is not None:
                g1, j1 = b1 % 4, b1 // 4
                hp = hh % HPR
                qrows = pl.ds(_mo((g1 * 8 + hh) * DH, DH), DH)
                parts = [qT_s[qrows, pl.ds(_mo(j1 * TQ, TQ), TQ)], jnp.zeros((DH * (7 - hp), TQ), BF16)]
                if hp > 0:
                    parts.insert(0, jnp.zeros((DH * hp, TQ), BF16))
                qm = jnp.concatenate(parts, axis=0)
                onehot = (lax.broadcasted_iota(jnp.int32, (DH, 8, 128), 2)
                          == lax.broadcasted_iota(jnp.int32, (DH, 8, 128), 0) + hh * DH)

            def v_item(idx):
                i, r = items[idx]
                zz = lax.shift_right_logical(b1, 5 + idx % 26)
                kf = kf_s[pl.ds(g1 + zz, 1), i, r:r + 8, :]
                kb = jnp.sum(jnp.where(onehot, kf, 0.0), axis=2, keepdims=True)
                qd = qb_s[pl.ds(j1 + zz, 1), qrows][0]
                sv = jnp.sum(kb * qd, axis=0)
                r0 = (i + 1) * CK - VMAX + r
                s_s[hh, r0:r0 + 8, :] = sv
                return sv

            tot_rg = (S - sum(vr)) // 8
            rg_done = 0
            vdone = 0
            for i in range(NC):
                sl = slice(i * CK, (i + 1) * CK)
                n = hh * NC + i
                if pieces is not None and n * npx // (8 * NC) != (n + 1) * npx // (8 * NC):
                    next(pieces)
                if b2 is not None:
                    sp = s_s[hh, sl, :].reshape(CK // 8, 8, TQ)
                    p = jnp.exp2(sp - mb[None]).reshape(CK, TQ)
                    for r in range(CK // 8 - 1, -1, -1):
                        pr = p[r * 8:(r + 1) * 8, :]
                        l8 = pr if l8 is None else l8 + pr
                    a = jnp.dot(vT_s[hrows, sl], p, preferred_element_type=F32)
                    acc = a if acc is None else a + acc
                if b1 is not None:
                    lo, hi = i * CK, (i + 1) * CK - vr[i]
                    kr = pltpu.bitcast(k_s[hh // HPR, pl.ds(g1, 1), lo // 2:hi // 2, :][0], BF16)
                    sT = jnp.dot(kr, qm, preferred_element_type=F32)
                    s_s[hh, lo:hi, :] = sT
                    for r in range((hi - lo) // 8):
                        sr = sT[r * 8:(r + 1) * 8, :]
                        m8 = sr if m8 is None else jnp.maximum(m8, sr)
                        rg_done += 1
                        want = nf + rg_done * (len(items) - nf - nl) // tot_rg + (nl if rg_done == tot_rg else 0)
                        while vdone < want and (b2 is None or items[vdone][0] <= i):
                            m8 = jnp.maximum(m8, v_item(vdone))
                            vdone += 1
            if b2 is not None:
                l = jnp.sum(l8, axis=0, keepdims=True)
                oT_s[hrows, pl.ds(_mo(j2 * TQ, TQ), TQ)] = (acc * (1.0 / l)).astype(BF16)
            if b1 is not None:
                assert vdone == len(items)
                m_s[hh] = jnp.max(m8, axis=0, keepdims=True)

        def c1_pieces(rb, first):
            rows = slice(rb * TM, (rb + 1) * TM)
            o = oT_s[:, rows].T
            cols = []
            for c in range(D // 128):
                cols.append(jnp.dot(o, wo_ref[:, c * 128:(c + 1) * 128], preferred_element_type=F32))
                if c == D // 128 - 1:
                    x1 = x_in(first, rows) + jnp.concatenate(cols, axis=1)
                    x_s[rows, :] = x1
                    xn_s[rows, :] = _ln(x1).astype(BF16)
                yield

        def c2_pieces(rb):
            rows = slice(rb * TM, (rb + 1) * TM)
            y = None
            hs = []
            for f in range(F // 128):
                fs = slice(f * 128, (f + 1) * 128)
                g = jnp.dot(xn_s[rows, :], wg_ref[:, fs], preferred_element_type=F32)
                yield
                u = jnp.dot(xn_s[rows, :], wu_ref[:, fs], preferred_element_type=F32)
                hs.append((g * u).astype(BF16))
                yield
                if f >= 1:
                    a = jnp.dot(hs[f - 1], wd_ref[(f - 1) * 128:f * 128, :], preferred_element_type=F32)
                    y = a if y is None else a + y
                    yield
            a = jnp.dot(hs[-1], wd_ref[F - 128:F, :], preferred_element_type=F32)
            y = x_s[rows, :] + (a + y)
            x_s[rows, :] = y
            out_s[rows, :] = y.astype(BF16)
            yield

        def c2(t):
            rows = pl.ds(_mo(t * TM, TM), TM)
            xn = xn_s[rows, :]
            g = jnp.dot(xn, wg_ref[...], preferred_element_type=F32)
            u = jnp.dot(xn, wu_ref[...], preferred_element_type=F32)
            hh = (g * u).astype(BF16)
            y = x_s[rows, :] + jnp.dot(hh, wd_ref[...], preferred_element_type=F32)
            x_s[rows, :] = y
            out_s[rows, :] = y.astype(BF16)

        def layer(li, carry):
            first = li == 0
            last = li == 1
            phase_a(first, li < 2)

            @pl.when(li >= 0)
            def _():
                for hh in range(8):
                    att_unit(lax.shift_right_logical(li, 1), None, hh, pattern0)

            def body(b, c):
                att_unit(b + 1, b, 0, pattern_first, nf=2)
                for hh in range(1, 7):
                    att_unit(b + 1, b, hh, pattern)
                att_unit(b + 1, b, 7, pattern_last, nl=2)
                return c
            lax.fori_loop(0, NB - 1, body, 0)

            @pl.when(first)
            def _():
                for i in range(4):
                    w_copy(i).wait()

            n1 = (S - TQ) // TM
            pieces = _chain(*[c1_pieces(rb, first) for rb in range(n1)], c2_pieces(0), c2_pieces(1))
            for hh in range(8):
                att_unit(None, NB - 1, hh, pattern, pieces)
            for n, _ in enumerate(pieces):
                if n == c1pos:
                    for _ in _chain(*[c1_pieces(rb, first) for rb in range(n1, NCT)]):
                        pass

            @pl.when(last)
            def _():
                o_copy(0).start()
                o_copy(1).start()

            def cbody(t, c):
                piece = jnp.minimum(t - 2, TQ // 128 - 1)
                prow = pl.ds(pl.multiple_of(piece * 128, 128), 128)
                xa_s[prow, :] = _ln(x_s[prow, :]).astype(BF16)
                c2(t)

                @pl.when(last)
                def _():
                    o_copy(t).start()
                return c
            lax.fori_loop(2, NCT, cbody, 0)
            return carry

        lax.fori_loop(0, 2, layer, 0)
        for t in range(NCT):
            o_copy(t).wait()

    @jax.jit
    def run(A_x, A_wqkv, A_wo, B_x, B_w_gate, B_w_up, B_w_down):
        x = A_x.reshape(S, D)
        out = pl.pallas_call(
            kernel,
            out_shape=jax.ShapeDtypeStruct((S, D), A_x.dtype),
            in_specs=[pl.BlockSpec(memory_space=pl.ANY)] * 6,
            out_specs=pl.BlockSpec(memory_space=pl.ANY),
            scratch_shapes=[
                pltpu.VMEM((S, D), BF16),
                pltpu.VMEM((D, 3 * D), BF16),
                pltpu.VMEM((D, D), BF16),
                pltpu.VMEM((D, F), BF16),
                pltpu.VMEM((D, F), BF16),
                pltpu.VMEM((F, D), BF16),
                pltpu.VMEM((S, D), BF16),
                pltpu.VMEM((S, D), F32),
                pltpu.VMEM((TQ, D), BF16),
                pltpu.VMEM((S, D), BF16),
                pltpu.VMEM((2 * D, D), BF16),
                pltpu.VMEM((NROT, 4, S // 2, 128), jnp.uint32),
                pltpu.VMEM((4, NC, VMAX, 128), F32),
                pltpu.VMEM((D, S), BF16),
                pltpu.VMEM((NA, D, 8, TQ), F32),
                pltpu.VMEM((D, S), F32),
                pltpu.VMEM((D, S), BF16),
                pltpu.VMEM((8, S, TQ), F32),
                pltpu.VMEM((8, 1, TQ), F32),
                pltpu.SemaphoreType.DMA((6,)),
                pltpu.SemaphoreType.DMA((4,)),
                pltpu.SemaphoreType.DMA((NCT,)),
            ],
            compiler_params=pltpu.CompilerParams(vmem_limit_bytes=120 * 1024 * 1024),
        )(x, A_wqkv, A_wo, B_w_gate, B_w_up, B_w_down)
        return out.reshape(1, S, D)
    return run


_run = _make()


def pallas_interleave_layers__softmax_full_mha__glu_gated_bilinear__prompt_kernel(
    A_x, A_wqkv, A_wo, B_x, B_w_gate, B_w_up, B_w_down
):
    return _run(A_x, A_wqkv, A_wo, B_x, B_w_gate, B_w_up, B_w_down)
```

```python
import math

import jax
import jax.numpy as jnp
from jax import lax
import jax.experimental.pallas as pl
import jax.experimental.pallas.tpu as pltpu

S, D, H, DH, F = 2048, 512, 32, 16, 1792
EPS = 1e-5
BF16 = jnp.bfloat16
F32 = jnp.float32
TQ = 512
CK = 128
NC = S // CK
NB = (H // 8) * (S // TQ)
NA = S // TQ
NROT = 4
HPR = 8 // NROT
QSCALE = (DH ** -0.5) * math.log2(math.e)

PATTERN = "1111111111110000"
PATTERN_FIRST = "2111111111110000"
PATTERN_LAST = "1111111111111000"
KV_A = (544, 416)
KV_C = 1280
MS1 = (64, 64)
RP = 304
MS2 = (64, 64, 64)
TT = 128
R0 = sum(MS1)
R2 = R0 + 4 * RP
assert R2 + sum(MS2) == S - TQ
OUT_TILES = ([(0, R0)] + [(R0 + i * RP, RP) for i in range(4)] + [(R2, S - TQ - R2)]
             + [(S - TQ + i * TT, TT) for i in range(TQ // TT)])


def _ln(x):
    m = jnp.mean(x, axis=-1, keepdims=True)
    xc = x - m
    v = jnp.mean(xc * xc, axis=-1, keepdims=True)
    return xc * lax.rsqrt(v + EPS)


def _mo(v, m):
    return v if isinstance(v, int) else pl.multiple_of(v, m)


def _chain(*gens):
    for g in gens:
        yield from g


def _kernel(x_hbm, wqkv_hbm, wo_hbm, wg_hbm, wu_hbm, wd_hbm, o_hbm,
            xin_s, wqkv_s, wo_s, wg_s, wu_s, wd_s, out_s,
            x_s, xa_s, xn_s, wqvT_s, k_s, kf_s, qT_s, qb_s, qb0_s, vT_s, oT_s, s_s, m_s,
            sem_x, sem_w, sem_o):
    def x_copy(t):
        rows = slice(t * TQ, (t + 1) * TQ) if t < 2 else slice(2 * TQ, S)
        return pltpu.make_async_copy(x_hbm.at[rows, :], xin_s.at[rows, :], sem_x.at[t])

    def wqkv_copy(i):
        cols = slice(i * D, (i + 1) * D)
        return pltpu.make_async_copy(wqkv_hbm.at[:, cols], wqkv_s.at[:, cols], sem_x.at[3 + i])

    w_pairs = ((wo_hbm, wo_s), (wg_hbm, wg_s), (wu_hbm, wu_s), (wd_hbm, wd_s))

    def w_copy(i):
        return pltpu.make_async_copy(w_pairs[i][0], w_pairs[i][1], sem_w.at[i])

    def o_copy(i, r0, n):
        rows = pl.ds(r0, n)
        return pltpu.make_async_copy(out_s.at[rows, :], o_hbm.at[rows, :], sem_o.at[i])

    x_copy(0).start()
    wqkv_copy(1).start()
    x_s[...] = jnp.zeros(x_s.shape, F32)
    x_copy(0).wait()
    wqkv_copy(0).start()
    wqkv_copy(2).start()
    xa_s[...] = _ln(xin_s[0:TQ, :].astype(F32)).astype(BF16)
    wqkv_copy(1).wait()
    x_copy(1).start()
    x_copy(2).start()

    def x_in(first, rows):
        return jnp.where(first, xin_s[rows, :].astype(F32), x_s[rows, :])

    def transpose_weights():
        wqT = wqkv_s[:, 0:D].astype(F32).T.astype(BF16)
        wvT = wqkv_s[:, 2 * D:3 * D].astype(F32).T.astype(BF16)
        for h in range(H):
            wqvT_s[2 * h * DH:(2 * h + 1) * DH, :] = wqT[h * DH:(h + 1) * DH]
            wqvT_s[(2 * h + 1) * DH:(2 * h + 2) * DH, :] = wvT[h * DH:(h + 1) * DH]

    def proj_k(t, xn):
        kk = jnp.dot(xn, wqkv_s[:, D:2 * D], preferred_element_type=F32)
        for g in range(4):
            kg = kk[:, g * 128:(g + 1) * 128]
            kf_s[g, t * TQ:(t + 1) * TQ, :] = kg
            ku = pltpu.bitcast(kg.astype(BF16), jnp.uint32)
            for r in range(NROT):
                k_s[r, g, t * TQ // 2:(t + 1) * TQ // 2, :] = (
                    ku if r == 0 else pltpu.roll(ku, 128 - r * HPR * DH, 1))

    def proj_qv(t, c, xn):
        cols = pl.ds(_mo(t * TQ + c * 128, 128), 128)
        qv = lax.dot_general(wqvT_s[...], xn, (((1,), (1,)), ((), ())), preferred_element_type=F32)
        qv = qv.reshape(H, 2 * DH, 128)
        q = qv[:, 0:DH, :].reshape(D, 128) * QSCALE
        qT_s[:, cols] = q.astype(BF16)
        q3 = q.reshape(D // 8, 8, 128)
        qrep = jnp.stack([jnp.broadcast_to(q3[:, s:s + 1, :], (D // 8, 8, 128)) for s in range(8)],
                         axis=1).reshape(D, 8, 128)
        qb_s[pl.ds(t, 1), :, :, pl.ds(_mo(c * 128, 128), 128)] = qrep[None]
        if isinstance(t, int) and t == 0:
            qb0_s[:, :, c * 128:(c + 1) * 128] = qrep[0:128]
        vT_s[:, cols] = qv[:, DH:2 * DH, :].reshape(D, 128)

    def qv_pieces(n0, cnt):
        for k in range(cnt):
            n = n0 + k
            proj_qv(n // 4, n % 4, xn_s[pl.ds(pl.multiple_of(n * 128, 128), 128), :])
            yield

    def phase_a(first):
        def ln_tile(t):
            rows = slice(t * TQ, (t + 1) * TQ)
            xn_s[rows, :] = _ln(x_in(first, rows)).astype(BF16)

        proj_k(0, xa_s[...])

        @pl.when(first)
        def _():
            wqkv_copy(0).wait()
            wqkv_copy(2).wait()
            transpose_weights()
            x_copy(1).wait()

        ln_tile(1)
        for c in range(3):
            proj_qv(0, c, xa_s[c * 128:(c + 1) * 128, :])

        @pl.when(first)
        def _():
            x_copy(2).wait()
            for i in range(4):
                w_copy(i).start()

        ln_tile(2)
        proj_k(1, xn_s[TQ:2 * TQ, :])
        ln_tile(3)
        proj_k(2, xn_s[2 * TQ:3 * TQ, :])
        proj_k(3, xn_s[3 * TQ:4 * TQ, :])
        proj_qv(0, 3, xa_s[3 * 128:4 * 128, :])

    def q_padded(b, hh, hp):
        g, j = b % 4, b // 4
        qrows = pl.ds(_mo((g * 8 + hh) * DH, DH), DH)
        parts = [qT_s[qrows, pl.ds(_mo(j * TQ, TQ), TQ)], jnp.zeros((DH * (7 - hp), TQ), BF16)]
        if hp > 0:
            parts.insert(0, jnp.zeros((DH * hp, TQ), BF16))
        return jnp.concatenate(parts, axis=0)

    def head_lanes(hh):
        return (lax.broadcasted_iota(jnp.int32, (DH, 8, 128), 2)
                == lax.broadcasted_iota(jnp.int32, (DH, 8, 128), 0) + hh * DH)

    def vpu_scores(kf, onehot, qd):
        kb = jnp.sum(jnp.where(onehot, kf, 0.0), axis=2, keepdims=True)
        return jnp.sum(kb * qd, axis=0)

    def att_unit(b1, b2, hh, pat=PATTERN, nf=0, nl=0, pieces=None, npx=0, done=None):
        g2, j2 = b2 % 4, b2 // 4
        mb = jnp.broadcast_to(m_s[hh], (8, TQ))
        hrows = pl.ds(_mo((g2 * 8 + hh) * DH, DH), DH)
        l8 = None
        acc = None
        if b1 is not None:
            vr = [16 * int(ch) for ch in pat]
            items = [(i, (i + 1) * CK - vr[i] + r) for i in range(NC) for r in range(0, vr[i], 8)]
            g1, j1 = b1 % 4, b1 // 4
            qrows = pl.ds(_mo((g1 * 8 + hh) * DH, DH), DH)
            qm = q_padded(b1, hh, hh % HPR)
            onehot = head_lanes(hh)
            tot_rg = (S - sum(vr)) // 8
            rg_done = 0
            vdone = 0
            m8 = None
        for i in range(NC):
            sl = slice(i * CK, (i + 1) * CK)
            while pieces is not None and done[0] < (hh * NC + i) * npx // (8 * NC - 1):
                next(pieces)
                done[0] += 1
            sp = s_s[hh, sl, :].reshape(CK // 8, 8, TQ)
            p = jnp.exp2(sp - mb[None]).reshape(CK, TQ)
            for r in range(CK // 8 - 1, -1, -1):
                pr = p[r * 8:(r + 1) * 8, :]
                l8 = pr if l8 is None else l8 + pr
            a = jnp.dot(vT_s[hrows, sl], p, preferred_element_type=F32)
            acc = a if acc is None else a + acc
            if b1 is not None:
                lo, hi = i * CK, (i + 1) * CK - vr[i]
                kr = pltpu.bitcast(k_s[hh // HPR, pl.ds(g1, 1), lo // 2:hi // 2, :][0], BF16)
                sT = jnp.dot(kr, qm, preferred_element_type=F32)
                s_s[hh, lo:hi, :] = sT
                for r in range((hi - lo) // 8):
                    sr = sT[r * 8:(r + 1) * 8, :]
                    m8 = sr if m8 is None else jnp.maximum(m8, sr)
                    rg_done += 1
                    want = nf + rg_done * (len(items) - nf - nl) // tot_rg + (nl if rg_done == tot_rg else 0)
                    while vdone < want and items[vdone][0] <= i:
                        r0 = items[vdone][1]
                        zz = lax.shift_right_logical(b1, 5 + vdone % 26)
                        sv = vpu_scores(kf_s[pl.ds(g1 + zz, 1), r0:r0 + 8, :], onehot,
                                        qb_s[pl.ds(j1 + zz, 1), qrows][0])
                        s_s[hh, r0:r0 + 8, :] = sv
                        m8 = jnp.maximum(m8, sv)
                        vdone += 1
        l = jnp.sum(l8, axis=0, keepdims=True)
        oT_s[hrows, pl.ds(_mo(j2 * TQ, TQ), TQ)] = (acc * (1.0 / l)).astype(BF16)
        if b1 is not None:
            assert vdone == len(items)
            m_s[hh] = jnp.max(m8, axis=0, keepdims=True)

    def hosted_pass1(b1, pair, hp, qm, kv, chunk, pieces, npieces, plen):
        g1, j1 = b1 % 4, b1 // 4
        hh = pair * HPR + hp
        qrows = pl.ds(pl.multiple_of((g1 * 8 + hh) * DH, DH), DH)
        onehot = head_lanes(hh)
        km = S - kv
        nch = -(-km // chunk)
        tot = km + npieces * plen
        now = 0
        vdone = 0
        pdone = 0
        m8 = None
        for c in range(nch):
            while pdone < (c + 1) * npieces // nch:
                next(pieces)
                pdone += 1
                now += plen
            lo, hi = c * chunk, min((c + 1) * chunk, km)
            kr = pltpu.bitcast(k_s[pl.ds(pair, 1), g1, lo // 2:hi // 2, :][0], BF16)
            sT = jnp.dot(kr, qm, preferred_element_type=F32)
            s_s[pl.ds(hh, 1), lo:hi, :] = sT[None]
            for r in range((hi - lo) // 8):
                sr = sT[r * 8:(r + 1) * 8, :]
                m8 = sr if m8 is None else jnp.maximum(m8, sr)
                now += 8
                while vdone < now * (kv // 8) // tot:
                    r0 = km + vdone * 8
                    zz = lax.shift_right_logical(pair, 5 + vdone % 26)
                    if b1 == 0:
                        qd = qb0_s[pl.ds(hh * DH + zz, DH)]
                    else:
                        qd = qb_s[pl.ds(j1 + zz, 1), qrows][0]
                    sv = vpu_scores(kf_s[g1:g1 + 1, r0:r0 + 8, :], onehot, qd)
                    s_s[pl.ds(hh, 1), r0:r0 + 8, :] = sv[None]
                    m8 = jnp.maximum(m8, sv)
                    vdone += 1
        assert vdone == kv // 8 and pdone == npieces
        m_s[pl.ds(hh, 1)] = jnp.max(m8, axis=0, keepdims=True)[None]

    def mixed(b, c):
        att_unit(b + 1, b, 0, PATTERN_FIRST, nf=2)
        for hh in range(1, 7):
            att_unit(b + 1, b, hh)
        att_unit(b + 1, b, 7, PATTERN_LAST, nl=2)
        return c

    def drain(b, pieces, npx, after):
        done = [0]
        for hh in range(8):
            att_unit(None, b, hh, pieces=pieces, npx=npx, done=done)
        next(pieces, None)
        for _ in _chain(after, pieces):
            pass

    def wo_pieces(r0, first, m):
        o = oT_s[:, r0:r0 + 256].T
        for s in range(256 // m):
            rows = slice(r0 + s * m, r0 + (s + 1) * m)
            cols = []
            for c in range(D // 128):
                cols.append(jnp.dot(o[s * m:(s + 1) * m], wo_s[:, c * 128:(c + 1) * 128],
                                    preferred_element_type=F32))
                if c == D // 128 - 1:
                    x1 = x_in(first, rows) + jnp.concatenate(cols, axis=1)
                    x_s[rows, :] = x1
                    xn_s[rows, :] = _ln(x1).astype(BF16)
                yield

    def ffn_pieces(row_groups, fw):
        n = len(row_groups)
        y = [None] * n
        hs = [None] * n
        xns = [xn_s[rows, :] for rows in row_groups] if fw > 128 else None
        for f in range(F // fw + 1):
            fs = slice(f * fw, (f + 1) * fw)
            for s, rows in enumerate(row_groups):
                hprev = hs[s]
                if f < F // fw:
                    g = jnp.dot(xns[s] if xns else xn_s[rows, :], wg_s[:, fs], preferred_element_type=F32)
                    yield
                    u = jnp.dot(xns[s] if xns else xn_s[rows, :], wu_s[:, fs], preferred_element_type=F32)
                    hs[s] = (g * u).astype(BF16)
                    yield
                if f >= 1:
                    a = jnp.dot(hprev, wd_s[(f - 1) * fw:f * fw, :], preferred_element_type=F32)
                    y[s] = a if y[s] is None else a + y[s]
                    if f == F // fw:
                        yy = x_s[rows, :] + y[s]
                        x_s[rows, :] = yy
                        out_s[rows, :] = yy.astype(BF16)
                    yield

    def groups(base, sizes):
        return [slice(base + sum(sizes[:s]), base + sum(sizes[:s + 1])) for s in range(len(sizes))]

    def layer(li, carry):
        first = li == 0
        last = li == 1

        def start_out(i, r0, n):
            @pl.when(last)
            def _():
                o_copy(i, r0, n).start()

        phase_a(first)

        def host_a(i, c):
            qm0, qm1 = q_padded(0, i * HPR, 0), q_padded(0, i * HPR + 1, 1)
            pieces = qv_pieces(4 + 3 * i, 3)
            hosted_pass1(0, i, 0, qm0, KV_A[0], 128, pieces, 2, 2 * D)
            hosted_pass1(0, i, 1, qm1, KV_A[1], 128, pieces, 1, 2 * D)
            return c
        lax.fori_loop(0, NROT, host_a, 0)

        lax.fori_loop(0, NB - 2, mixed, 0)

        @pl.when(first)
        def _():
            for i in range(4):
                w_copy(i).wait()

        drain(NB - 2, _chain(*[wo_pieces(r0, first, 128) for r0 in range(0, S - TQ, 256)],
                             ffn_pieces(groups(0, MS1), 128)), 127, ())
        start_out(0, 0, R0)

        def host_c(i, c):
            r0 = pl.multiple_of(R0 + i * RP, 16)
            pieces = ffn_pieces([pl.ds(r0, RP)], F // 2)
            for hp in range(HPR):
                hosted_pass1(NB - 1, i, hp, q_padded(NB - 1, i * HPR + hp, hp), KV_C, 256, pieces, 3, RP * 7)
            start_out(i + 1, r0, RP)
            return c
        lax.fori_loop(0, NROT, host_c, 0)

        drain(NB - 1, ffn_pieces(groups(R2, MS2), 128), 122,
              _chain(wo_pieces(S - TQ, first, 256), wo_pieces(S - 256, first, 256)))
        start_out(5, R2, S - TQ - R2)

        def tail(t, c):
            prow = pl.ds(pl.multiple_of(t * TT, TT), TT)
            xa_s[prow, :] = _ln(x_s[prow, :]).astype(BF16)
            r0 = pl.multiple_of(S - TQ + t * TT, TT)
            for _ in ffn_pieces([pl.ds(r0, TT)], F):
                pass
            start_out(6 + t, r0, TT)
            return c
        lax.fori_loop(0, TQ // TT, tail, 0)
        return carry

    lax.fori_loop(0, 2, layer, 0)
    for i, (r0, n) in enumerate(OUT_TILES):
        o_copy(i, r0, n).wait()


@jax.jit
def pallas_interleave_layers__softmax_full_mha__glu_gated_bilinear__prompt_kernel(
    A_x, A_wqkv, A_wo, B_x, B_w_gate, B_w_up, B_w_down
):
    out = pl.pallas_call(
        _kernel,
        out_shape=jax.ShapeDtypeStruct((S, D), A_x.dtype),
        in_specs=[pl.BlockSpec(memory_space=pl.ANY)] * 6,
        out_specs=pl.BlockSpec(memory_space=pl.ANY),
        scratch_shapes=[
            pltpu.VMEM((S, D), BF16),
            pltpu.VMEM((D, 3 * D), BF16),
            pltpu.VMEM((D, D), BF16),
            pltpu.VMEM((D, F), BF16),
            pltpu.VMEM((D, F), BF16),
            pltpu.VMEM((F, D), BF16),
            pltpu.VMEM((S, D), BF16),
            pltpu.VMEM((S, D), F32),
            pltpu.VMEM((TQ, D), BF16),
            pltpu.VMEM((S, D), BF16),
            pltpu.VMEM((2 * D, D), BF16),
            pltpu.VMEM((NROT, 4, S // 2, 128), jnp.uint32),
            pltpu.VMEM((4, S, 128), F32),
            pltpu.VMEM((D, S), BF16),
            pltpu.VMEM((NA, D, 8, TQ), F32),
            pltpu.VMEM((128, 8, TQ), F32),
            pltpu.VMEM((D, S), F32),
            pltpu.VMEM((D, S), BF16),
            pltpu.VMEM((8, S, TQ), F32),
            pltpu.VMEM((8, 1, TQ), F32),
            pltpu.SemaphoreType.DMA((6,)),
            pltpu.SemaphoreType.DMA((4,)),
            pltpu.SemaphoreType.DMA((len(OUT_TILES),)),
        ],
        compiler_params=pltpu.CompilerParams(vmem_limit_bytes=120 * 1024 * 1024),
    )(A_x.reshape(S, D), A_wqkv, A_wo, B_w_gate, B_w_up, B_w_down)
    return out.reshape(1, S, D)
```
